```python
import os as _os
_os.environ.setdefault("JAX_PLATFORMS", "cpu")
import jax
import jax.numpy as jnp

def _softmax(x, axis=-1):
    return jax.nn.softmax(x, axis=axis)
def _gelu(x):
    return jax.nn.gelu(x, approximate=True)
def _silu(x):
    return jax.nn.silu(x)
def _sigmoid(x):
    return jax.nn.sigmoid(x)
def _layernorm(x, axis=-1, eps=1e-5):
    m = jnp.mean(x, axis=axis, keepdims=True)
    v = jnp.var(x, axis=axis, keepdims=True)
    return (x - m) / jnp.sqrt(v + eps)
def _scatter_add(tgt, idx, src, axis=0):
    return tgt.at[idx].add(src)
def _segment_sum(src, seg, n):
    return jax.ops.segment_sum(src, seg, n)
class _Rng:
    def __init__(self, key):
        self._k = key
    def _next(self):
        self._k, sub = jax.random.split(self._k)
        return sub
    def normal(self, shape):
        return jax.random.normal(self._next(), shape, dtype=jnp.bfloat16)
    def randint(self, lo, hi, shape):
        return jax.random.randint(self._next(), shape, lo, hi, dtype=jnp.int32)
    def uniform(self, shape, lo=0.0, hi=1.0):
        return jax.random.uniform(self._next(), shape, jnp.bfloat16, lo, hi)
    def permutation(self, n):
        return jax.random.permutation(self._next(), n)


kernel_name = 'concat_heads__linear_attn_block__ssm_conv_s5__prompt'

def setup_inputs():
    _rng = _Rng(jax.random.key(int.from_bytes(__import__("os").urandom(4), "little")))
    _w = (lambda a: (lambda t: t.astype(jnp.bfloat16) if jnp.issubdtype(t.dtype, jnp.floating) else t)(jnp.asarray(a)))
    def _A_setup():
        B, S, D = 1, 2048, 640
        return {
            "x": _w((lambda *s: _rng.normal(s) * 0.05)(B, S, D)),
            "wqkv": _w((lambda *s: _rng.normal(s) * 0.8)(D, 3 * D)),
            "wo": _w((lambda *s: _rng.normal(s) * 0.05)(D, D)),
        }
    _A_in = _A_setup()

    def _B_setup():
        B, S, D = 1, 2048, 640
        P = D
        Lambda_re = -0.5 * jnp.exp((lambda *s: _rng.normal(s) * 0.4)(P))
        Lambda_im = (lambda *s: _rng.normal(s) * 0.4)(P) * 1.0
        B_re = (lambda *s: _rng.normal(s) * 0.4)(P, D) * (D ** -0.5)
        B_im = (lambda *s: _rng.normal(s) * 0.4)(P, D) * (D ** -0.5)
        C_re = (lambda *s: _rng.normal(s) * 0.4)(D, P) * (P ** -0.5)
        C_im = (lambda *s: _rng.normal(s) * 0.4)(D, P) * (P ** -0.5)
        log_dt = (lambda *s: _rng.normal(s) * 0.4)(P) * 0.3 - 2.0
        Dskip = (lambda *s: _rng.normal(s) * 0.4)(D)
        return {
            "x": _w((lambda *s: _rng.normal(s) * 0.05)(B, S, D)),
            "Lambda_re": _w(Lambda_re),
            "Lambda_im": _w(Lambda_im),
            "B_re": _w(B_re),
            "B_im": _w(B_im),
            "C_re": _w(C_re),
            "C_im": _w(C_im),
            "log_dt": _w(log_dt),
            "Dskip": _w(Dskip),
        }
    _B_in = _B_setup()

    return {
        "A_x": _A_in["x"],
        "A_wqkv": _A_in["wqkv"],
        "A_wo": _A_in["wo"],
        "B_x": _B_in["x"],
        "B_Lambda_re": _B_in["Lambda_re"],
        "B_Lambda_im": _B_in["Lambda_im"],
        "B_B_re": _B_in["B_re"],
        "B_B_im": _B_in["B_im"],
        "B_C_re": _B_in["C_re"],
        "B_C_im": _B_in["C_im"],
        "B_log_dt": _B_in["log_dt"],
        "B_Dskip": _B_in["Dskip"],
    }

def reference(A_x, A_wqkv, A_wo, B_x, B_Lambda_re, B_Lambda_im, B_B_re, B_B_im, B_C_re, B_C_im, B_log_dt, B_Dskip):
    def _A_ref(x, wqkv, wo):
        B, S, D = x.shape
        H = 32; Dh = D // H
        qkv = (lambda x, *d: x.transpose(*d))((x @ wqkv).reshape(B, S, 3, H, Dh), 2, 0, 3, 1, 4)
        q, k, v = qkv[0], qkv[1], qkv[2]
        phi = lambda t: jnp.where(t > 0, t + 1, jnp.exp(t)) + 1e-6
        pq, pk = phi(q), phi(k)
        kv = jnp.einsum("bhsd,bhse->bhde", pk, v)
        z = jnp.einsum("bhsd->bhd", pk)
        num = jnp.einsum("bhqd,bhde->bhqe", pq, kv)
        den = jnp.einsum("bhqd,bhd->bhq", pq, z)[..., None] + 1e-6
        o = num / den
        return (lambda x, *d: x.transpose(*d))(o, 0, 2, 1, 3).reshape(B, S, D) @ wo

    def _B_ref(x, Lambda_re, Lambda_im, B_re, B_im, C_re, C_im, log_dt, Dskip):
        Bsz, L, H = x.shape
        Lam = Lambda_re + 1j * Lambda_im
        Bmat = B_re + 1j * B_im
        Cmat = C_re + 1j * C_im
        dt = jnp.exp(log_dt)
        Lam_bar = jnp.exp(dt * Lam)
        B_bar = ((Lam_bar - 1.0) / Lam)[:, None] * Bmat
        Bu = jnp.einsum("bld,pd->blp", x + 0j, B_bar)
        h = jnp.zeros_like(Bu[:, 0, :])
        hs = []
        for t in range(L):
            h = Lam_bar[None, :] * h + Bu[:, t, :]
            hs.append(h)
        hseq = jnp.stack(hs, 1)
        y = 2.0 * jnp.einsum("blp,dp->bld", hseq, Cmat).real + x * Dskip[None, None, :]
        return y

    a = _A_ref(A_x, A_wqkv, A_wo)
    b = _B_ref(B_x, B_Lambda_re, B_Lambda_im, B_B_re, B_B_im, B_C_re, B_C_im, B_log_dt, B_Dskip)
    return jnp.concatenate([a, b], axis=-1)
```

```python
import jax
import jax.numpy as jnp
from jax import lax
from jax.experimental import pallas as pl
from jax.experimental.pallas import tpu as pltpu

S = 2048
D = 640
NL = 5
H = 32
DH = 20
TB = 256
SEGS = (20, 12)
BASES = (0, 8 * SEGS[0])

F32 = jnp.float32
BF16 = jnp.bfloat16
NT = (((1,), (1,)), ((), ()))

T_LR, T_LI, T_D, T_CR, T_CI, T_NCI = 0, 1, 2, 3, 4, 25
def _tab_idx(sub, k, part):
    return 5 + sub * 10 + k * 2 + part
NTAB = 5 + 20 + 1

SCOPES = False
QB = 256


def _cmul(ar, ai, br, bi):
    return ar * br - ai * bi, ar * bi + ai * br


def _phi(t):
    return jnp.where(t > 0, t + 1.0, jnp.exp(t)) + 1e-6


U32 = jnp.uint32


def _pk(x):
    return pltpu.bitcast(x.astype(BF16), U32)


def _up(x):
    return pltpu.bitcast(x, BF16)


def _lt(x, lt):
    return x[:, lt * 128:(lt + 1) * 128]


def _kernel(xa_hbm, wqkv_hbm, wo_hbm, xb_hbm, lre_hbm, lim_hbm, bre_hbm, bim_hbm,
            cre_hbm, cim_hbm, ldt_hbm, dsk_hbm,
            out_hbm,
            xa, xb, wq, wk, wv, wo, bcat, cre, cim, ccat, wkT, wqT, slab, slab2, tab,
            xs, xp, hb, ys, oa, gacc, zacc, kvs, mp, zrow, carry_ref,
            v_lre, v_lim, v_ldt, v_dsk, sem_in, sem_out):
    def scope(name):
        return jax.named_scope(name)

    groups = {}
    def cp(g, src, dst):
        c = pltpu.make_async_copy(src, dst, sem_in.at[g])
        c.start()
        groups.setdefault(g, []).append(c)
    def cp_rows(g, src, dst, r0, n, d0=None):
        d0 = r0 if d0 is None else d0
        cp(g, src.at[pl.ds(r0, n), :], dst.at[pl.ds(d0, n), :])
    def wait(g):
        if SCOPES:
            with scope("wait%d" % g):
                for c in groups[g]:
                    c.wait()
        else:
            for c in groups[g]:
                c.wait()
    def cp_pair(g, p):
        cp_rows(g, bre_hbm, bcat, p * 128, 128, p * 256)
        cp_rows(g, bim_hbm, bcat, p * 128, 128, p * 256 + 128)
    xb_h = xb_hbm.at[0]
    xa_h = xa_hbm.at[0]

    def it_copies(i):
        a0 = i * 512
        t0 = 1024 + i * TB
        if not isinstance(i, int):
            a0 = pl.multiple_of(a0, 512)
            t0 = pl.multiple_of(t0, TB)
        return (pltpu.make_async_copy(xa_h.at[pl.ds(a0, 512), :], xa.at[pl.ds(a0, 512), :], sem_in.at[7 + i]),
                pltpu.make_async_copy(xb_h.at[pl.ds(t0, TB), :], xb.at[pl.ds(t0, TB), :], sem_in.at[7 + i]))

    cp(6, lre_hbm, v_lre); cp(6, lim_hbm, v_lim); cp(6, ldt_hbm, v_ldt); cp(6, dsk_hbm, v_dsk)
    cp_rows(0, xb_h, xb, 0, 512)
    cp_rows(1, bre_hbm, bcat, 0, 256)
    cp_rows(2, bim_hbm, bcat, 0, 256, D)
    cp_rows(2, bre_hbm, bcat, 256, 256)
    cp_rows(3, bim_hbm, bcat, 256, 384, D + 256)
    cp_rows(3, bre_hbm, bcat, 512, 128)
    cp_rows(3, xb_h, xb, 512, 512)
    cp(4, wqkv_hbm.at[:, pl.ds(D, D)], wk)
    cp(4, cre_hbm, cre)
    cp(4, cim_hbm, cim)
    for i in range(4):
        for c in it_copies(i):
            c.start()
    cp(5, wqkv_hbm.at[:, pl.ds(0, D)], wq)
    cp(5, wqkv_hbm.at[:, pl.ds(2 * D, D)], wv)
    cp(5, wo_hbm, wo)

    def out_b(t0, lt):
        return pltpu.make_async_copy(
            ys.at[lt, pl.ds(t0, TB), :],
            out_hbm.at[0, pl.ds(t0, TB), pl.ds(D + lt * 128, 128)], sem_out.at[0])

    def out_a(a0, n):
        return pltpu.make_async_copy(
            oa.at[pl.ds(a0, n), :], out_hbm.at[0, pl.ds(a0, n), pl.ds(0, D)], sem_out.at[0])

    def half(t0):
        return t0 // 2 if isinstance(t0, int) else pl.multiple_of(t0 // 2, TB // 2)

    def b_prep(r0):
        xf = xb[pl.ds(r0, TB), :].astype(F32)
        for lt in range(NL):
            xs[lt, pl.ds(r0, TB), :] = _lt(xf, lt)
        rows = []
        for base, n in zip(BASES, SEGS):
            for j in range(n):
                rows.append(jnp.concatenate(
                    [xs[lt, pl.ds(r0 + base + j, 8, stride=n), :] for lt in range(NL)], axis=1))
        return jnp.concatenate(rows, axis=0).astype(BF16)

    def b_bu(x, tiles):
        w = jnp.concatenate([bcat[t * 128:(t + 1) * 128, :] for t in tiles], axis=0)
        r = lax.dot_general(x, w, NT, preferred_element_type=F32)
        return {t: _lt(r, i) for i, t in enumerate(tiles)}

    carry = {}
    def b_scan(items):
        sub8 = lax.broadcasted_iota(jnp.int32, (8, 128), 0)
        chains = []
        for bu, t0, lt in items:
            for c in range(bu[0].shape[0] // TB):
                for si in range(2):
                    chains.append((bu, c * TB + BASES[si], si, lt, t0))
        lam = {lt: (tab[T_LR, :, lt * 128:(lt + 1) * 128], tab[T_LI, :, lt * 128:(lt + 1) * 128])
               for _, _, lt in items}
        tb = lambda si, k, lt: (tab[_tab_idx(si, k, 0), :, lt * 128:(lt + 1) * 128],
                                tab[_tab_idx(si, k, 1), :, lt * 128:(lt + 1) * 128])
        ld = lambda bu, r: (bu[0][r:r + 8, :], bu[1][r:r + 8, :])

        def step(h, a, b):
            return (a[0] * h[0] - a[1] * h[1] + b[0], a[0] * h[1] + a[1] * h[0] + b[1])
        st = [ld(bu, o) for bu, o, si, lt, t0 in chains]
        for j in range(1, max(SEGS)):
            for ix, (bu, o, si, lt, t0) in enumerate(chains):
                if j < SEGS[si]:
                    st[ix] = step(st[ix], lam[lt], ld(bu, o + 8 * j))
        for k in range(3):
            for ix, (bu, o, si, lt, t0) in enumerate(chains):
                e = st[ix]
                sh = (pltpu.roll(e[0], 1 << k, 0), pltpu.roll(e[1], 1 << k, 0))
                st[ix] = step(sh, tb(si, k, lt), e)
        hin = []
        for ix, (bu, o, si, lt, t0) in enumerate(chains):
            e = st[ix]
            rl = tuple(jnp.where(sub8 == 0, 0.0, pltpu.roll(v, 1, 0)) for v in e)
            lb = tuple(jnp.broadcast_to(v[7:8, :], (8, 128)) for v in e)
            prev = carry.get(lt)
            if prev is None:
                hin.append(rl)
                carry[lt] = lb
            else:
                hin.append(step(prev, tb(si, 3, lt), rl))
                carry[lt] = step(prev, tb(si, 4, lt), lb)
        st = hin
        for j in range(0, max(SEGS), 2):
            for ix, (bu, o, si, lt, t0) in enumerate(chains):
                if j < SEGS[si]:
                    r = o + 8 * j
                    h1 = step(st[ix], lam[lt], ld(bu, r))
                    h2 = step(h1, lam[lt], ld(bu, r + 8))
                    st[ix] = h2
                    rows = pl.ds(half(t0) + r // 2, 8)
                    hb[rows, lt * 128:(lt + 1) * 128] = _pk(jnp.concatenate([h1[0], h2[0]], axis=0))
                    hb[rows, D + lt * 128:D + (lt + 1) * 128] = _pk(jnp.concatenate([h1[1], h2[1]], axis=0))

    def carry_save():
        for lt in range(NL):
            carry_ref[0, :, lt * 128:(lt + 1) * 128] = carry[lt][0]
            carry_ref[1, :, lt * 128:(lt + 1) * 128] = carry[lt][1]

    def carry_load():
        for lt in range(NL):
            carry[lt] = (carry_ref[0, :, lt * 128:(lt + 1) * 128],
                         carry_ref[1, :, lt * 128:(lt + 1) * 128])

    def b_y_store(t0, y, lt):
        dv = tab[T_D, :, lt * 128:(lt + 1) * 128]
        for base, n in zip(BASES, SEGS):
            for j in range(n):
                r = base + 8 * j
                idx = pl.ds(t0 + base + j, 8, stride=n)
                ys[lt, idx, :] = y[r:r + 8, :] + xs[lt, idx, :] * dv
        out_b(t0, lt).start()

    def b_y(t0, l0=0, l1=NL):
        h = _up(hb[pl.ds(half(t0), TB // 2), :])
        y = lax.dot_general(h, _up(ccat[l0 * 64:l1 * 64, :]), NT, preferred_element_type=F32)
        for lt in range(l0, l1):
            b_y_store(t0, _lt(y, lt - l0), lt)

    def tables():
        lre = v_lre[...].astype(F32).reshape(1, D)
        lim = v_lim[...].astype(F32).reshape(1, D)
        dt = jnp.exp(v_ldt[...].astype(F32).reshape(1, D)).astype(BF16).astype(F32)
        dsk = v_dsk[...].astype(F32).reshape(1, D)
        mag = jnp.exp(dt * lre)
        ang = dt * lim
        lbr = mag * jnp.cos(ang)
        lbi = mag * jnp.sin(ang)
        sc = jnp.maximum(jnp.abs(lre), jnp.abs(lim))
        a_ = lre / sc
        b_ = lim / sc
        dn = (a_ * a_ + b_ * b_) * sc
        nr = lbr - 1.0
        cr = (nr * a_ + lbi * b_) / dn
        ci = (lbi * a_ - nr * b_) / dn
        bc = lambda v: jnp.broadcast_to(v, (8, D))
        sub = lax.broadcasted_iota(jnp.int32, (8, D), 0)
        tab[T_LR] = bc(lbr)
        tab[T_LI] = bc(lbi)
        tab[T_D] = bc(dsk)
        tab[T_CR] = bc(2.0 * cr)
        tab[T_CI] = bc(2.0 * ci)
        tab[T_NCI] = bc(-2.0 * ci)
        pw = [(lbr, lbi)]
        for _ in range(5):
            pw.append(_cmul(*pw[-1], *pw[-1]))
        for si, n in enumerate(SEGS):
            acc = None
            for b in range(6):
                if (n >> b) & 1:
                    acc = pw[b] if acc is None else _cmul(*acc, *pw[b])
            w = (jnp.ones((8, D), F32), jnp.zeros((8, D), F32))
            for k in range(3):
                a8 = (bc(acc[0]), bc(acc[1]))
                tab[_tab_idx(si, k, 0)] = jnp.where(sub >= (1 << k), a8[0], 0.0)
                tab[_tab_idx(si, k, 1)] = jnp.where(sub >= (1 << k), a8[1], 0.0)
                wm = _cmul(*w, *a8)
                bit = ((sub >> k) & 1) == 1
                w = (jnp.where(bit, wm[0], w[0]), jnp.where(bit, wm[1], w[1]))
                acc = _cmul(*acc, *acc)
            tab[_tab_idx(si, 3, 0)] = w[0]
            tab[_tab_idx(si, 3, 1)] = w[1]
            tab[_tab_idx(si, 4, 0)] = bc(acc[0])
            tab[_tab_idx(si, 4, 1)] = bc(acc[1])

    def c_prep(l0=0, l1=NL):
        for r in range(l0 * 128, l1 * 128, 16):
            for lt in range(NL):
                cs = slice(lt * 128, (lt + 1) * 128)
                c_r = cre[r:r + 16, cs].astype(F32)
                c_i = cim[r:r + 16, cs].astype(F32)
                cr2 = tab[T_CR, 0:1, cs]
                ci2 = tab[T_CI, 0:1, cs]
                nci2 = tab[T_NCI, 0:1, cs]
                ccat[r // 2:r // 2 + 8, cs] = _pk(c_r * cr2 - c_i * ci2)
                ccat[r // 2:r // 2 + 8, D + lt * 128:D + (lt + 1) * 128] = _pk(c_r * nci2 - c_i * cr2)

    def wk_prep():
        for j in range(NL):
            wkT[j * 64:(j + 1) * 64, :] = _pk(wk[:, j * 128:(j + 1) * 128].astype(F32).T)

    def a_kT(a0, n):
        xc = xa[pl.ds(a0, n), :]
        kT = lax.dot_general(_up(wkT[...]), xc, NT, preferred_element_type=F32)
        pk = _phi(kT)
        zs = zacc[...]
        for q in range(n // 128):
            zs = zs + _lt(pk, q)
        zacc[...] = zs
        return pk.astype(BF16)

    def a_G(pk, a0, n):
        xc = xa[pl.ds(a0, n), :]
        gacc[...] += jnp.dot(pk, xc, preferred_element_type=F32)

    rng = ((0, 144), (112, 272), (240, 400), (368, 528), (496, 640))

    def a_kv():
        for j, (lo, hi) in enumerate(rng):
            g = gacc[lo:hi, :].astype(BF16)
            kv = jnp.dot(g, wv[:, j * 128:(j + 1) * 128], preferred_element_type=F32)
            rh = (lax.broadcasted_iota(jnp.int32, kv.shape, 0) + lo) // DH
            ch = (lax.broadcasted_iota(jnp.int32, kv.shape, 1) + j * 128) // DH
            kvs[j, 0:(hi - lo) // 2, :] = _pk(jnp.where(rh == ch, kv, 0.0))

    def a_M():
        parts = [jnp.dot(_up(kvs[j, 0:(hi - lo) // 2, :]), wo[j * 128:(j + 1) * 128, :],
                         preferred_element_type=F32) for j, (lo, hi) in enumerate(rng)]
        pieces = []
        pos = 0
        for j, (lo, hi) in enumerate(rng):
            nxt = rng[j + 1][0] if j + 1 < len(rng) else hi
            pieces.append(parts[j][pos - lo:nxt - lo])
            if j + 1 < len(rng):
                pieces.append(parts[j][nxt - lo:hi - lo] + parts[j + 1][0:hi - nxt])
                pos = hi
        m = jnp.concatenate(pieces, axis=0)
        for lt in range(NL):
            slab[lt] = _lt(m, lt)

    def a_mp():
        for d in range(DH):
            for lt in range(NL):
                mp[d * 16:(d + 1) * 16, lt * 128:(lt + 1) * 128] = _pk(
                    slab[lt, pl.ds(d, H, stride=DH), :])

    def a_z():
        zp = jnp.concatenate([zacc[pl.ds(d, H, stride=DH), :] for d in range(DH)], axis=0)
        zhi = zp.astype(BF16)
        zlo = (zp - zhi.astype(F32)).astype(BF16)
        ones = jnp.ones((8, 128), BF16)
        zrow[...] = (lax.dot_general(ones, zhi, NT, preferred_element_type=F32)
                     + lax.dot_general(ones, zlo, NT, preferred_element_type=F32))

    def a_wq():
        for lt in range(NL):
            slab2[lt] = wq[lt * 128:(lt + 1) * 128, :].astype(F32).T
            for d in range(DH):
                wqT[d * 16:(d + 1) * 16, lt * 128:(lt + 1) * 128] = _pk(
                    slab2[lt, pl.ds(d, H, stride=DH), :])

    def a_q(a0, n):
        outs = []
        for b in range(n // QB):
            xc = xa[pl.ds(a0 + b * QB, QB), :]
            q = lax.dot_general(xc, _up(wqT[...]), NT, preferred_element_type=F32)
            pq = _phi(q)
            zr = zrow[0:1, :]
            t = _lt(pq, 0) * _lt(zr, 0)
            for lt in range(1, NL):
                t = t + _lt(pq, lt) * _lt(zr, lt)
            t = t + pltpu.roll(t, 64, 1)
            t = t + pltpu.roll(t, 32, 1)
            r = 1.0 / (t + 1e-6)
            outs.append(jnp.concatenate([_lt(pq, lt) * r for lt in range(NL)], axis=1).astype(BF16))
        return jnp.concatenate(outs, axis=0)

    def a_o(pqn, a0, n):
        oa[pl.ds(a0, n), :] = jnp.dot(pqn, _up(mp[...]), preferred_element_type=F32)
        out_a(a0, n).start()

    gacc[...] = jnp.zeros(gacc.shape, F32)
    zacc[...] = jnp.zeros(zacc.shape, F32)
    wait(6)
    tables()
    wait(0)
    xp[0:128] = _pk(b_prep(0))
    xp[128:256] = _pk(b_prep(256))
    x0 = lambda: _up(xp[0:256])
    x1 = lambda: _up(xp[256:512])
    u = {}
    def bu0(tiles):
        for t, v in b_bu(x0(), tiles).items():
            u[(0, t)] = v
    def bu1(tiles):
        for t, v in b_bu(x1(), tiles).items():
            u[(512, t)] = v
    def sc(lst):
        b_scan([((u.pop((t0, p)), u.pop((t0, p + 5))), t0, p) for t0, p in lst])
    wait(1)
    bu0([0, 1])
    wait(2)
    bu0([5, 6])
    sc([(0, 0), (0, 1)])
    bu0([2, 3])
    wait(3)
    bu0([7, 8])
    sc([(0, 2), (0, 3)])
    bu0([4, 9])
    sc([(0, 4)])
    xp[256:384] = _pk(b_prep(512))
    xp[384:512] = _pk(b_prep(768))
    bu1([0, 5])
    sc([(512, 0)])
    bu1([1, 2])
    wait(4)
    bu1([6, 7])
    sc([(512, 1), (512, 2)])
    c_prep(0, 1)
    b_y(0, 0, 1)
    bu1([3, 8])
    sc([(512, 3)])
    c_prep(1, 2)
    b_y(0, 1, 2)
    bu1([4, 9])
    sc([(512, 4)])
    carry_save()
    c_prep(2, 5)
    b_y(0, 2, 5)
    wk_prep()

    def loop_a(i, c):
        for cc in it_copies(i):
            cc.wait()
        a0 = pl.multiple_of(i * 512, 512)
        tb0 = pl.multiple_of(1024 + i * TB, TB)
        ty = pl.multiple_of((i + 1) * TB, TB)
        pk = a_kT(a0, 512)
        x = b_prep(tb0)
        uu = b_bu(x, [0, 5, 1, 6, 2, 7, 3, 8, 4, 9])
        carry_load()
        b_scan([((uu[p], uu[p + 5]), tb0, p) for p in range(5)])
        carry_save()
        a_G(pk, a0, 512)
        b_y(ty)
        return c
    with scope("LA"):
        lax.fori_loop(0, 4, loop_a, 0)

    wait(5)
    a_kv()
    a_z()
    a_M()
    b_y(5 * TB)
    a_mp()
    a_wq()

    def loop_b(i, c):
        a0 = pl.multiple_of(i * 1024, 1024)
        t0 = pl.multiple_of((i + 6) * TB, TB)
        p0 = a_q(a0, 256)
        p1 = a_q(a0 + 256, 256)
        a_o(p0, a0, 256)
        p2 = a_q(a0 + 512, 256)
        a_o(p1, a0 + 256, 256)
        p3 = a_q(a0 + 768, 256)
        a_o(p2, a0 + 512, 256)
        b_y(t0, 0, 2)
        a_o(p3, a0 + 768, 256)
        b_y(t0, 2, 3)
        b_y(t0, 3, 4)
        b_y(t0, 4, 5)
        return c
    with scope("LB"):
        lax.fori_loop(0, 2, loop_b, 0)

    with scope("wait_out"):
        for c in range(8):
            for lt in range(NL):
                out_b(c * TB, lt).wait()
        for i in range(8):
            out_a(i * 256, 256).wait()


@jax.jit
def pallas_concat_heads__linear_attn_block__ssm_conv_s5__prompt_kernel(A_x, A_wqkv, A_wo, B_x, B_Lambda_re, B_Lambda_im, B_B_re, B_B_im,
              B_C_re, B_C_im, B_log_dt, B_Dskip):
    any_spec = pl.BlockSpec(memory_space=pl.ANY)
    V = pltpu.VMEM
    return pl.pallas_call(
        _kernel,
        out_shape=jax.ShapeDtypeStruct((1, S, 2 * D), F32),
        in_specs=[any_spec] * 12,
        out_specs=any_spec,
        scratch_shapes=[
            V((S, D), BF16),
            V((S, D), BF16),
            V((D, D), BF16),
            V((D, D), BF16),
            V((D, D), BF16),
            V((D, D), BF16),
            V((2 * D, D), BF16),
            V((D, D), BF16),
            V((D, D), BF16),
            V((D // 2, 2 * D), U32),
            V((D // 2, D), U32),
            V((D // 2, D), U32),
            V((NL, D, 128), F32),
            V((NL, D, 128), F32),
            V((NTAB, 8, D), F32),
            V((NL, S, 128), F32),
            V((512, D), U32),
            V((S // 2, 2 * D), U32),
            V((NL, S, 128), F32),
            V((S, D), F32),
            V((D, D), F32),
            V((D, 128), F32),
            V((NL, 80, 128), U32),
            V((D // 2, D), U32),
            V((8, D), F32),
            V((2, 8, D), F32),
            V((D,), BF16), V((D,), BF16), V((D,), BF16), V((D,), BF16),
            pltpu.SemaphoreType.DMA((11,)),
            pltpu.SemaphoreType.DMA((1,)),
        ],
        compiler_params=pltpu.CompilerParams(vmem_limit_bytes=110 * 1024 * 1024),
    )(A_x, A_wqkv, A_wo, B_x, B_Lambda_re, B_Lambda_im, B_B_re, B_B_im,
      B_C_re, B_C_im, B_log_dt, B_Dskip)
```

```python
import jax
import jax.numpy as jnp
from jax import lax
from jax.experimental import pallas as pl
from jax.experimental.pallas import tpu as pltpu

S = 2048
D = 640
NL = 5
H = 32
DH = 20
TB = 256
SEGS = (20, 12)
BASES = (0, 8 * SEGS[0])
NB = 32

F32 = jnp.float32
BF16 = jnp.bfloat16
U32 = jnp.uint32
NT = (((1,), (1,)), ((), ()))

T_LR, T_LI, T_D, T_CR, T_CI, T_NCI = 0, 1, 2, 3, 4, 5


def _tab_idx(sub, k, part):
    return 6 + sub * 8 + k * 2 + part


NTAB = 6 + 16

ORD = (2, 3, 1, 0, 5, 4, 6)
ORDK = (2, 4, 3, 0, 6, 1, 5)
ORDG = (2, 3, 4, 1, 0, 5, 6)
ORDY0 = (1, 4, 0, 3, 6, 2, 5)

KTOP = ((0, 128), (256, 384), (512, 576))
KBOT = ((128, 256), (384, 512), (576, 640))
KVR = ((0, 144), (112, 272), (240, 400), (368, 528), (496, 640))


def _cmul(ar, ai, br, bi):
    return ar * br - ai * bi, ar * bi + ai * br


def _phi(t):
    return jnp.where(t > 0, t + 1.0, jnp.exp(t)) + 1e-6


def _pk(x):
    return pltpu.bitcast(x.astype(BF16), U32)


def _up(x):
    return pltpu.bitcast(x, BF16)


def _sums_a(a11, a12, a21, a22):
    return [a11 + a22, a21 + a22, a11, a22, a11 + a12, a21 - a11, a12 - a22]


def _op_b(i, g):
    return [lambda: g(0, 0) + g(1, 1), lambda: g(0, 0), lambda: g(0, 1) - g(1, 1),
            lambda: g(1, 0) - g(0, 0), lambda: g(1, 1), lambda: g(0, 0) + g(0, 1),
            lambda: g(1, 0) + g(1, 1)][i]()


def _combine(m):
    return (m[0] + m[3] - m[4] + m[6], m[2] + m[4], m[1] + m[3], m[0] - m[1] + m[2] + m[5])


def _lt(x, lt):
    return x[:, lt * 128:(lt + 1) * 128]


def _dot_nt(a, b):
    return lax.dot_general(a, b, NT, preferred_element_type=F32)


def _dot(a, b):
    return jnp.dot(a, b, preferred_element_type=F32)


def _kernel(xa_hbm, wqkv_hbm, wo_hbm, xb_hbm, lre_hbm, lim_hbm, bre_hbm, bim_hbm,
            cre_hbm, cim_hbm, ldt_hbm, dsk_hbm,
            out_hbm,
            xa, xb, xw, wq, wk, wv, wo, bcat, cre, cim, cS, cR, slab, slab2, tab,
            xp, hb, ys, oa, gM, gR, zacc, kvs, mS, mKR, mNR, zrow, carry_ref, pqs,
            wkS, wkR, wqS, wqKR, wqNR, xS, xpS, bS, rrs, gb,
            v_lre, v_lim, v_ldt, v_dsk, sem_in, sem_out):
    groups = {}

    def cp(g, src, dst):
        c = pltpu.make_async_copy(src, dst, sem_in.at[g])
        c.start()
        groups.setdefault(g, []).append(c)

    def cp_rows(g, src, dst, r0, n, d0=None):
        d0 = r0 if d0 is None else d0
        cp(g, src.at[pl.ds(r0, n), :], dst.at[pl.ds(d0, n), :])

    def wait(g):
        for c in groups[g]:
            c.wait()

    xb_h = xb_hbm.at[0]
    xa_h = xa_hbm.at[0]

    def it_copies(i):
        a0 = i * 512
        t0 = 1024 + i * TB
        if not isinstance(i, int):
            a0 = pl.multiple_of(a0, 512)
            t0 = pl.multiple_of(t0, TB)
        return (pltpu.make_async_copy(xa_h.at[pl.ds(a0, 512), :], xa.at[pl.ds(a0, 512), :],
                                      sem_in.at[7 + i]),
                pltpu.make_async_copy(xb_h.at[pl.ds(t0, TB), :], xb.at[pl.ds(t0, TB), :],
                                      sem_in.at[7 + i]))

    cp(6, lre_hbm, v_lre)
    cp(6, lim_hbm, v_lim)
    cp(6, ldt_hbm, v_ldt)
    cp(6, dsk_hbm, v_dsk)
    cp_rows(0, xb_h, xb, 0, 512)
    cp_rows(1, bre_hbm, bcat, 0, 256)
    cp_rows(2, bim_hbm, bcat, 0, 256, D)
    cp_rows(2, bre_hbm, bcat, 256, 256)
    cp_rows(3, bim_hbm, bcat, 256, 384, D + 256)
    cp_rows(3, bre_hbm, bcat, 512, 128)
    cp_rows(3, xb_h, xb, 512, 512)
    cp(4, wqkv_hbm.at[:, pl.ds(D, D)], wk)
    cp(4, cre_hbm, cre)
    cp(4, cim_hbm, cim)
    cp(4, wqkv_hbm.at[:, pl.ds(0, D)], wq)
    for i in range(4):
        for c in it_copies(i):
            c.start()
    cp(5, wqkv_hbm.at[:, pl.ds(2 * D, D)], wv)
    cp(5, wo_hbm, wo)

    def out_b(t0, lt):
        return pltpu.make_async_copy(
            ys.at[lt, pl.ds(t0, TB), :],
            out_hbm.at[0, pl.ds(t0, TB), pl.ds(D + lt * 128, 128)], sem_out.at[0])

    def out_a(a0, n):
        return pltpu.make_async_copy(
            oa.at[pl.ds(a0, n), :], out_hbm.at[0, pl.ds(a0, n), pl.ds(0, D)], sem_out.at[0])

    frac = {}

    def chunk(c):
        t0 = pl.multiple_of(c * TB, TB)
        frac[id(t0)] = (pl.multiple_of(c * (TB // 2), TB // 2), pl.multiple_of(c * (TB // 4), TB // 4))
        return t0

    def half(t0):
        return t0 // 2 if isinstance(t0, int) else frac[id(t0)][0]

    def quarter(t0):
        return t0 // 4 if isinstance(t0, int) else frac[id(t0)][1]

    def b_stage(r0):
        for lt in range(NL):
            xw[pl.ds(lt * (S // 2) + half(r0), TB // 2), :] = pltpu.bitcast(
                xb[pl.ds(r0, TB), lt * 128:(lt + 1) * 128], U32)

    def b_ld2(r0, g, lt):
        si = 0 if g < SEGS[0] else 1
        j = g - (0 if si == 0 else SEGS[0])
        w = xw[pl.ds(lt * (S // 2) + half(r0) + (BASES[si] + j) // 2, 8, stride=SEGS[si] // 2), :]
        lo = pltpu.bitcast(w << 16, F32)
        hi = pltpu.bitcast(w & jnp.uint32(0xFFFF0000), F32)
        return jnp.concatenate([lo, hi], axis=0)

    def b_prep(r0):
        for g in range(0, 32, 2):
            for lt in range(NL):
                xp[r0 // 2 + 4 * g:r0 // 2 + 4 * g + 8, lt * 128:(lt + 1) * 128] = _pk(b_ld2(r0, g, lt))

    def b_prep_s(tops, bots):
        for k in range(len(tops)):
            tl = [b_ld2(*tops[k], lt) for lt in range(NL)]
            bl = [b_ld2(*bots[k], lt) for lt in range(NL)]
            for c in range(2):
                for i, v in enumerate(_sums_a(tl[c], tl[2 + c], bl[c], bl[2 + c])):
                    xpS[8 * k:8 * k + 8, i * 256 + c * 128:i * 256 + (c + 1) * 128] = _pk(v)
            xpS[8 * k:8 * k + 8, 1792:1920] = _pk(tl[4])
            xpS[8 * k:8 * k + 8, 1920:2048] = _pk(bl[4])
        return 16 * len(tops)

    def bs_op(p, i):
        if i in (1, 4):
            return
        for r in range(p * 128, (p + 1) * 128, 32):
            for c in range(2):
                g = lambda kh, nh: bcat[nh * D + r:nh * D + r + 32,
                                        (2 * kh + c) * 128:(2 * kh + c + 1) * 128].astype(F32)
                bS[i * 320 + r // 2:i * 320 + r // 2 + 16, c * 128:(c + 1) * 128] = _pk(_op_b(i, g))

    def bu_prod(hn, p, i):
        if i == 1:
            w = bcat[p * 128:(p + 1) * 128, 0:256]
        elif i == 4:
            w = bcat[D + p * 128:D + (p + 1) * 128, 256:512]
        else:
            w = _up(bS[i * 320 + p * 64:i * 320 + (p + 1) * 64, :])
        return _dot_nt(_up(xpS[0:hn // 2, i * 256:(i + 1) * 256]), w)

    def bu_rem(hn, p):
        xr = jnp.concatenate([_up(xpS[0:hn // 2, 1792:1920]), _up(xpS[0:hn // 2, 1920:2048])], axis=0)
        w = jnp.concatenate([bcat[p * 128:(p + 1) * 128, 512:640],
                             bcat[D + p * 128:D + (p + 1) * 128, 512:640]], axis=0)
        return _dot_nt(xr, w)

    def bu_fin(m, rem):
        c11, c12, c21, c22 = _combine(m)
        return (jnp.concatenate([c11, c21], axis=0) + rem[:, 0:128],
                jnp.concatenate([c12, c22], axis=0) + rem[:, 128:256])

    def bu_plain(x, tiles):
        w = jnp.concatenate([bcat[t * 128:(t + 1) * 128, :] for t in tiles], axis=0)
        r = _dot_nt(x, w)
        return {t: _lt(r, i) for i, t in enumerate(tiles)}

    carry = {}

    def b_scan(items):
        sub8 = lax.broadcasted_iota(jnp.int32, (8, 128), 0)
        chains = []
        for bu, t0, lt in items:
            for c in range(bu[0].shape[0] // TB):
                for si in range(2):
                    chains.append((bu, c * TB + BASES[si], si, lt, t0))
        lam = {lt: (tab[T_LR, :, lt * 128:(lt + 1) * 128], tab[T_LI, :, lt * 128:(lt + 1) * 128])
               for _, _, lt in items}
        tb = lambda si, k, lt: (tab[_tab_idx(si, k, 0), :, lt * 128:(lt + 1) * 128],
                                tab[_tab_idx(si, k, 1), :, lt * 128:(lt + 1) * 128])
        ld = lambda bu, r: (bu[0][r:r + 8, :], bu[1][r:r + 8, :])

        def step(h, a, b):
            return (a[0] * h[0] - a[1] * h[1] + b[0], a[0] * h[1] + a[1] * h[0] + b[1])

        st = [ld(bu, o) for bu, o, si, lt, t0 in chains]
        for j in range(1, max(SEGS)):
            for ix, (bu, o, si, lt, t0) in enumerate(chains):
                if j < SEGS[si]:
                    st[ix] = step(st[ix], lam[lt], ld(bu, o + 8 * j))
        for k in range(3):
            for ix, (bu, o, si, lt, t0) in enumerate(chains):
                e = st[ix]
                sh = (pltpu.roll(e[0], 1 << k, 0), pltpu.roll(e[1], 1 << k, 0))
                st[ix] = step(sh, tb(si, k, lt), e)
        for ix, (bu, o, si, lt, t0) in enumerate(chains):
            rl = tuple(jnp.where(sub8 == 0, 0.0, pltpu.roll(v, 1, 0)) for v in st[ix])
            prev = carry.get(lt)
            h = rl if prev is None else step(prev, tb(si, 3, lt), rl)
            for j in range(0, SEGS[si], 4):
                r = o + 8 * j
                h1 = step(h, lam[lt], ld(bu, r))
                h2 = step(h1, lam[lt], ld(bu, r + 8))
                h3 = step(h2, lam[lt], ld(bu, r + 16))
                h = step(h3, lam[lt], ld(bu, r + 24))
                cat = lambda a, b: jnp.concatenate([a, b], axis=0)
                a11, a12 = cat(h1[0], h2[0]), cat(h1[1], h2[1])
                a21, a22 = cat(h3[0], h[0]), cat(h3[1], h[1])
                sm = _sums_a(a11, a12, a21, a22)
                rows = pl.ds(quarter(t0) + r // 4, 8)
                for k, v in enumerate([a11, a12, a21, a22, sm[0], sm[1], sm[4], sm[5], sm[6]]):
                    hb[rows, k * D + lt * 128:k * D + (lt + 1) * 128] = _pk(v)
            carry[lt] = tuple(jnp.broadcast_to(v[7:8, :], (8, 128)) for v in h)

    def carry_save():
        for lt in range(NL):
            carry_ref[0, :, lt * 128:(lt + 1) * 128] = carry[lt][0]
            carry_ref[1, :, lt * 128:(lt + 1) * 128] = carry[lt][1]

    def carry_load():
        for lt in range(NL):
            carry[lt] = (carry_ref[0, :, lt * 128:(lt + 1) * 128],
                         carry_ref[1, :, lt * 128:(lt + 1) * 128])

    def y_store(t0, ytop, ybot, lt):
        dv = tab[T_D, :, lt * 128:(lt + 1) * 128]
        for base, n in zip(BASES, SEGS):
            for j in range(0, n, 2):
                xv = b_ld2(t0, base // 8 + j, lt)
                r = (base + 8 * (j - j % 4)) // 2
                y = ytop if j % 4 < 2 else ybot
                for e in range(2):
                    idx = pl.ds(t0 + base + j + e, 8, stride=n)
                    ys[lt, idx, :] = y[r + 8 * e:r + 8 * e + 8, :] + xv[8 * e:8 * e + 8] * dv
        out_b(t0, lt).start()

    hidx = {0: 4, 1: 5, 2: 0, 3: 3, 4: 6, 5: 7, 6: 8}

    def y_main(t0, order=ORD):
        rows = pl.ds(quarter(t0), TB // 4)
        m = [None] * 7
        for i in order:
            m[i] = _dot_nt(_up(hb[rows, hidx[i] * D:(hidx[i] + 1) * D]),
                           _up(cS[i * 128:(i + 1) * 128, :]))
        c11, c12, c21, c22 = _combine(m)
        for c in range(2):
            y_store(t0, _lt(c12, c), _lt(c22, c), 2 + c)
        for c in range(2):
            y_store(t0, _lt(c11, c), _lt(c21, c), c)

    def y_rem(t0):
        rows = pl.ds(quarter(t0), TB // 4)
        h = jnp.concatenate([_up(hb[rows, 0:2 * D]), _up(hb[rows, 2 * D:4 * D])], axis=0)
        y = _dot_nt(h, _up(cR[...]))
        y_store(t0, y[0:128], y[128:256], 4)

    def tables():
        lre = v_lre[...].astype(F32).reshape(1, D)
        lim = v_lim[...].astype(F32).reshape(1, D)
        dt = jnp.exp(v_ldt[...].astype(F32).reshape(1, D)).astype(BF16).astype(F32)
        dsk = v_dsk[...].astype(F32).reshape(1, D)
        mag = jnp.exp(dt * lre)
        ang = dt * lim
        lbr = mag * jnp.cos(ang)
        lbi = mag * jnp.sin(ang)
        sc = jnp.maximum(jnp.abs(lre), jnp.abs(lim))
        a_ = lre / sc
        b_ = lim / sc
        dn = (a_ * a_ + b_ * b_) * sc
        nr = lbr - 1.0
        cr = (nr * a_ + lbi * b_) / dn
        ci = (lbi * a_ - nr * b_) / dn
        bc = lambda v: jnp.broadcast_to(v, (8, D))
        sub = lax.broadcasted_iota(jnp.int32, (8, D), 0)
        tab[T_LR] = bc(lbr)
        tab[T_LI] = bc(lbi)
        tab[T_D] = bc(dsk)
        tab[T_CR] = bc(2.0 * cr)
        tab[T_CI] = bc(2.0 * ci)
        tab[T_NCI] = bc(-2.0 * ci)
        pw = [(lbr, lbi)]
        for _ in range(4):
            pw.append(_cmul(*pw[-1], *pw[-1]))
        for si, n in enumerate(SEGS):
            acc = None
            for b in range(5):
                if (n >> b) & 1:
                    acc = pw[b] if acc is None else _cmul(*acc, *pw[b])
            w = (jnp.ones((8, D), F32), jnp.zeros((8, D), F32))
            for k in range(3):
                a8 = (bc(acc[0]), bc(acc[1]))
                tab[_tab_idx(si, k, 0)] = jnp.where(sub >= (1 << k), a8[0], 0.0)
                tab[_tab_idx(si, k, 1)] = jnp.where(sub >= (1 << k), a8[1], 0.0)
                wm = _cmul(*w, *a8)
                bit = ((sub >> k) & 1) == 1
                w = (jnp.where(bit, wm[0], w[0]), jnp.where(bit, wm[1], w[1]))
                if k < 2:
                    acc = _cmul(*acc, *acc)
            tab[_tab_idx(si, 3, 0)] = w[0]
            tab[_tab_idx(si, 3, 1)] = w[1]

    def c_prep():
        def pq(r, lt, which):
            cs = slice(lt * 128, (lt + 1) * 128)
            c_r = cre[r:r + 16, cs].astype(F32)
            c_i = cim[r:r + 16, cs].astype(F32)
            if which == 0:
                return c_r * tab[T_CR, 0:1, cs] - c_i * tab[T_CI, 0:1, cs]
            return c_r * tab[T_NCI, 0:1, cs] - c_i * tab[T_CR, 0:1, cs]

        def put(i, r, lt, v):
            cS[i * 128 + r // 2:i * 128 + r // 2 + 8, lt * 128:(lt + 1) * 128] = _pk(v)

        p1, q2 = {}, {}
        pos = [(r, lt) for r in range(0, 256, 16) for lt in range(NL)]
        for r, lt in pos:
            p1[r, lt] = pq(r, lt, 0)
            put(1, r, lt, p1[r, lt])
        for r, lt in pos:
            q2[r, lt] = pq(256 + r, lt, 1)
            put(4, r, lt, q2[r, lt])
            put(0, r, lt, p1[r, lt] + q2[r, lt])
        for r, lt in pos:
            q1 = pq(r, lt, 1)
            put(3, r, lt, q1 - p1[r, lt])
            put(6, r, lt, q1 + q2[r, lt])
        for r, lt in pos:
            p2 = pq(256 + r, lt, 0)
            put(2, r, lt, p2 - q2[r, lt])
            put(5, r, lt, p1[r, lt] + p2)
        for which in range(2):
            for r in range(0, 128, 16):
                for lt in range(NL):
                    cR[r // 2:r // 2 + 8, which * D + lt * 128:which * D + (lt + 1) * 128] = _pk(
                        pq(512 + r, lt, which))

    def wk_prep():
        blk = lambda kt, ft: wk[kt * 128:(kt + 1) * 128, ft * 128:(ft + 1) * 128].astype(F32)
        rnd = lambda v: v.astype(BF16).astype(F32)
        for i in ORDK:
            for fp in range(2):
                for c in range(2):
                    v = _op_b(i, lambda kh, nh: blk(2 * kh + c, 2 * fp + nh))
                    wkS[i * 160 + fp * 64:i * 160 + (fp + 1) * 64, c * 128:(c + 1) * 128] = _pk(rnd(v).T)
        for c in range(2):
            t = [blk(c, 4).T, blk(2 + c, 4).T]
            for i in range(7):
                v = _op_b(i, lambda kh, nh: t[kh][64 * nh:64 * (nh + 1)])
                wkS[i * 160 + 128:i * 160 + 160, c * 128:(c + 1) * 128] = _pk(v)
        pos = 0
        tr = [blk(4, ft).T for ft in range(NL)]
        for lo, hi in KTOP + KBOT:
            wkR[pos // 2:(pos + hi - lo) // 2, :] = _pk(tr[lo // 128][lo % 128:lo % 128 + hi - lo])
            pos += hi - lo

    def wq_transpose():
        for lt in range(NL):
            slab2[lt] = wq[lt * 128:(lt + 1) * 128, :].astype(F32).T

    def wq_ops():
        g = lambda d, lt: slab2[lt, pl.ds(d, H, stride=DH), :]
        for i in ORD:
            for d in range(8):
                for c in range(2):
                    v = _op_b(i, lambda kh, nh: g(d + 8 * nh, 2 * kh + c))
                    wqS[i * 128 + d * 16:i * 128 + (d + 1) * 16, c * 128:(c + 1) * 128] = _pk(v)
        for d in range(16):
            wqKR[d * 16:(d + 1) * 16, :] = _pk(g(d, 4))
        for d in range(16, 20):
            for lt in range(NL):
                wqNR[(d - 16) * 16:(d - 15) * 16, lt * 128:(lt + 1) * 128] = _pk(g(d, lt))

    xidx = {0: 0, 1: 1, 4: 2, 5: 3, 6: 4}

    def x_sums(a0):
        for r in range(0, 256, 32):
            for c in range(2):
                g = lambda ro, co: xa[pl.ds(a0 + ro + r, 32),
                                      (co + c) * 128:(co + c + 1) * 128].astype(F32)
                sm = _sums_a(g(0, 0), g(0, 2), g(256, 0), g(256, 2))
                for i, k in xidx.items():
                    xS[k * 128 + r // 2:k * 128 + r // 2 + 16, c * 128:(c + 1) * 128] = _pk(sm[i])

    def x_op(a0, i):
        if i == 2:
            return xa[pl.ds(a0, 256), 0:256]
        if i == 3:
            return xa[pl.ds(a0 + 256, 256), 256:512]
        return _up(xS[xidx[i] * 128:(xidx[i] + 1) * 128, :])

    def a_k(a0):
        rem = _dot_nt(_up(wkR[...]), xa[pl.ds(a0, 512), 512:640])
        m = [None] * 7
        for i in ORDK:
            m[i] = _dot_nt(_up(wkS[i * 160:(i + 1) * 160, :]), x_op(a0, i))
        c11, c12, c21, c22 = _combine(m)
        a11 = _phi(c11 + rem[0:320, 0:256])
        a12 = _phi(c21 + rem[0:320, 256:512])
        a21 = _phi(c12 + rem[320:640, 0:256])
        a22 = _phi(c22 + rem[320:640, 256:512])
        zt = (_lt(a11, 0) + _lt(a11, 1)) + (_lt(a12, 0) + _lt(a12, 1))
        zb = (_lt(a21, 0) + _lt(a21, 1)) + (_lt(a22, 0) + _lt(a22, 1))
        for zz, rngs in ((zt, KTOP), (zb, KBOT)):
            pos = 0
            for lo, hi in rngs:
                zacc[lo:hi, :] += zz[pos:pos + hi - lo]
                pos += hi - lo
        ops = [v.astype(BF16) for v in _sums_a(a11, a12, a21, a22)]
        full = jnp.concatenate([jnp.concatenate([ops[2], a12.astype(BF16)], axis=1),
                                jnp.concatenate([a21.astype(BF16), ops[3]], axis=1)], axis=0)
        return ops, full

    gmap = {0: 0, 1: 2, 2: 6, 3: 5, 4: 3, 5: 4, 6: 1}

    def a_q_nrem(a0):
        pqs[pl.ds(a0, 512), 512:640] = _phi(_dot_nt(xa[pl.ds(a0, 512), :], _up(wqNR[...])))

    def a_q(a0):
        rem = _dot_nt(xa[pl.ds(a0, 512), 512:640], _up(wqKR[...]))
        m = [None] * 7
        for i in ORDK:
            m[i] = _dot_nt(x_op(a0, i), _up(wqS[i * 128:(i + 1) * 128, :]))
        c11, c12, c21, c22 = _combine(m)
        pqs[pl.ds(a0, 256), 0:256] = _phi(c11 + rem[0:256, 0:256])
        pqs[pl.ds(a0, 256), 256:512] = _phi(c12 + rem[0:256, 256:512])
        pqs[pl.ds(a0 + 256, 256), 0:256] = _phi(c21 + rem[256:512, 0:256])
        pqs[pl.ds(a0 + 256, 256), 256:512] = _phi(c22 + rem[256:512, 256:512])

    def a_z():
        for lt in range(NL):
            zp = jnp.concatenate(
                [zacc[pl.ds(d, H, stride=DH), :] for d in range(4 * lt, 4 * lt + 4)], axis=0)
            zrow[:, lt * 128:(lt + 1) * 128] = jnp.broadcast_to(
                jnp.sum(zp.T, axis=0, keepdims=True), (8, 128))

    def g_pack(gm, gr):
        c11, c12, c21, c22 = _combine(gm)
        for top, (cl, cr_), rngs in ((0, (c11, c12), KTOP), (320, (c21, c22), KBOT)):
            pos = 0
            for lo, hi in rngs:
                gb[lo // 2:hi // 2, 0:256] = _pk(cl[pos:pos + hi - lo])
                gb[lo // 2:hi // 2, 256:512] = _pk(cr_[pos:pos + hi - lo])
                gb[lo // 2:hi // 2, 512:640] = _pk(gr[top + pos:top + pos + hi - lo])
                pos += hi - lo

    def a_kv():
        for j, (lo, hi) in enumerate(KVR):
            kv = _dot(_up(gb[lo // 2:hi // 2, :]), wv[:, j * 128:(j + 1) * 128])
            rh = (lax.broadcasted_iota(jnp.int32, kv.shape, 0) + lo) // DH
            ch = (lax.broadcasted_iota(jnp.int32, kv.shape, 1) + j * 128) // DH
            kvs[j * 80:j * 80 + (hi - lo) // 2, :] = _pk(jnp.where(rh == ch, kv, 0.0))

    def a_m():
        parts = [_dot(_up(kvs[j * 80:j * 80 + (hi - lo) // 2, :]), wo[j * 128:(j + 1) * 128, :])
                 for j, (lo, hi) in enumerate(KVR)]
        pieces = []
        pos = 0
        for j, (lo, hi) in enumerate(KVR):
            nxt = KVR[j + 1][0] if j + 1 < len(KVR) else hi
            pieces.append(parts[j][pos - lo:nxt - lo])
            if j + 1 < len(KVR):
                pieces.append(parts[j][nxt - lo:hi - lo] + parts[j + 1][0:hi - nxt])
                pos = hi
        m = jnp.concatenate(pieces, axis=0)
        for lt in range(NL):
            slab[lt] = _lt(m, lt)
        g = lambda d, lt: slab[lt, pl.ds(d, H, stride=DH), :]
        for i in ORD:
            for d in range(8):
                for c in range(2):
                    v = _op_b(i, lambda kh, nh: g(d + 8 * kh, 2 * nh + c))
                    mS[i * 128 + d * 16:i * 128 + (d + 1) * 16, c * 128:(c + 1) * 128] = _pk(v)
        for d in range(16, 20):
            for lt in range(4):
                mKR[(d - 16) * 16:(d - 15) * 16, lt * 128:(lt + 1) * 128] = _pk(g(d, lt))
        for d in range(DH):
            mNR[d * 16:(d + 1) * 16, :] = _pk(g(d, 4))

    def a_o(a0, n):
        hn = n // 2
        for r in range(a0, a0 + n, NB):
            t = pqs[r:r + NB, 0:128] * zrow[0:1, 0:128]
            for lt in range(1, NL):
                t = t + pqs[r:r + NB, lt * 128:(lt + 1) * 128] * zrow[0:1, lt * 128:(lt + 1) * 128]
            t = t + pltpu.roll(t, 64, 1)
            t = t + pltpu.roll(t, 32, 1)
            rrs[r:r + NB, :] = 1.0 / (t + 1e-6)

        def norm_rows(r):
            pq = pqs[r:r + NB, :]
            rr = rrs[r:r + NB, :]
            return jnp.concatenate([_lt(pq, lt) * rr for lt in range(NL)], axis=1)

        tops, bots, sums = [], [], [[] for _ in range(7)]
        for r in range(0, hn, NB):
            tp = norm_rows(a0 + r)
            bt = norm_rows(a0 + hn + r)
            sm = _sums_a(tp[:, 0:256], tp[:, 256:512], bt[:, 0:256], bt[:, 256:512])
            tops.append(tp.astype(BF16))
            bots.append(bt.astype(BF16))
            for i in (0, 1, 4, 5, 6):
                sums[i].append(sm[i].astype(BF16))
        full = jnp.concatenate(tops + bots, axis=0)
        ops = [None] * 7
        for i in (0, 1, 4, 5, 6):
            ops[i] = jnp.concatenate(sums[i], axis=0)
        ops[2] = full[0:hn, 0:256]
        ops[3] = full[hn:n, 256:512]
        oa[a0:a0 + n, 512:640] = _dot(full, _up(mNR[...]))
        rem = _dot(full[:, 512:640], _up(mKR[...]))
        m = [None] * 7
        for i in ORD:
            m[i] = _dot(ops[i], _up(mS[i * 128:(i + 1) * 128, :]))
        c11, c12, c21, c22 = _combine(m)
        oa[a0:a0 + hn, 0:256] = c11 + rem[0:hn, 0:256]
        oa[a0:a0 + hn, 256:512] = c12 + rem[0:hn, 256:512]
        oa[a0 + hn:a0 + n, 0:256] = c21 + rem[hn:n, 0:256]
        oa[a0 + hn:a0 + n, 256:512] = c22 + rem[hn:n, 256:512]
        out_a(a0, n).start()

    gM[...] = jnp.zeros(gM.shape, F32)
    gR[...] = jnp.zeros(gR.shape, F32)
    zacc[...] = jnp.zeros(zacc.shape, F32)
    wait(6)
    tables()
    wait(0)
    b_stage(0)
    b_stage(256)
    b_prep(0)
    b_prep(256)

    u = {}

    def sc(ps):
        b_scan([((u.pop(p), u.pop(p + 5)), 0, p) for p in ps])

    wait(1)
    ra = bu_plain(_up(xp[0:128]), [0, 1])
    rb = bu_plain(_up(xp[128:256]), [0, 1])
    u.update({t: jnp.concatenate([ra[t], rb[t]], axis=0) for t in (0, 1)})
    wait(2)
    u.update(bu_plain(_up(xp[...]), [5, 6]))
    sc([0, 1])
    u.update(bu_plain(_up(xp[...]), [2, 3]))
    wait(3)
    u.update(bu_plain(_up(xp[...]), [7, 8]))
    sc([2, 3])
    u.update(bu_plain(_up(xp[...]), [4, 9]))
    sc([4])

    b_stage(512)
    b_stage(768)
    hn = b_prep_s([(512, g) for g in range(0, 32, 2)], [(768, g) for g in range(0, 32, 2)])
    mt = {}

    def rem1(p):
        mt[p] = ([None] * 7, bu_rem(hn, p))

    def prod1(p, k0, k1):
        for k in range(k0, k1):
            bs_op(p, ORD[k])
            mt[p][0][ORD[k]] = bu_prod(hn, p, ORD[k])
        if k1 == 7:
            b_scan([(bu_fin(*mt[p]), 512, p)])

    rem1(0)
    rem1(1)
    rem1(2)
    prod1(0, 0, 7)
    prod1(1, 0, 7)
    prod1(2, 0, 7)
    rem1(3)
    prod1(3, 0, 3)
    wait(4)
    c_prep()
    prod1(3, 3, 5)
    rem1(4)
    y_main(0, ORDY0)
    prod1(3, 5, 7)
    prod1(4, 0, 7)
    y_main(TB)
    y_rem(0)
    y_rem(TB)
    carry_save()
    wk_prep()
    wq_transpose()

    def main(i, c):
        for cc in it_copies(i):
            cc.wait()
        a0 = pl.multiple_of(i * 512, 512)
        tb0 = chunk(i + 4)
        ty = chunk(i + 2)
        b_stage(tb0)
        x_sums(a0)
        wq_ops()
        y_rem(ty)
        ops, full = a_k(a0)
        a_q_nrem(a0)
        h2 = b_prep_s([(tb0, g) for g in range(0, 16, 2)], [(tb0, g) for g in range(16, 32, 2)])
        carry_load()
        for p in range(NL):
            rem = bu_rem(h2, p)
            m = [None] * 7
            for k in ORD:
                m[k] = bu_prod(h2, p, k)
            b_scan([(bu_fin(m, rem), tb0, p)])
        carry_save()
        gm = [None] * 7
        for k in ORDG:
            gm[k] = gM[k] + _dot(ops[k], x_op(a0, gmap[k]))
            gM[k] = gm[k]
        a_q(a0)
        y_main(ty)
        gr = gR[...] + _dot(full, xa[pl.ds(a0, 512), 512:640])
        gR[...] = gr
        g_pack(gm, gr)
        a_z()
        return c

    lax.fori_loop(0, 4, main, 0)

    wait(5)
    a_kv()
    y_main(6 * TB)
    a_m()
    y_rem(6 * TB)
    for i in range(8):
        a_o(i * 256, 256)
    y_main(7 * TB)
    y_rem(7 * TB)

    for c in range(8):
        for lt in range(NL):
            out_b(c * TB, lt).wait()
    for i in range(8):
        out_a(i * 256, 256).wait()


@jax.jit
def pallas_concat_heads__linear_attn_block__ssm_conv_s5__prompt_kernel(
    A_x: jax.Array,
    A_wqkv: jax.Array,
    A_wo: jax.Array,
    B_x: jax.Array,
    B_Lambda_re: jax.Array,
    B_Lambda_im: jax.Array,
    B_B_re: jax.Array,
    B_B_im: jax.Array,
    B_C_re: jax.Array,
    B_C_im: jax.Array,
    B_log_dt: jax.Array,
    B_Dskip: jax.Array,
):
    any_spec = pl.BlockSpec(memory_space=pl.ANY)
    V = pltpu.VMEM
    return pl.pallas_call(
        _kernel,
        out_shape=jax.ShapeDtypeStruct((1, S, 2 * D), F32),
        in_specs=[any_spec] * 12,
        out_specs=any_spec,
        scratch_shapes=[
            V((S, D), BF16),
            V((S, D), BF16),
            V((NL * (S // 2), 128), U32),
            V((D, D), BF16),
            V((D, D), BF16),
            V((D, D), BF16),
            V((D, D), BF16),
            V((2 * D, D), BF16),
            V((D, D), BF16),
            V((D, D), BF16),
            V((7 * 128, D), U32),
            V((64, 2 * D), U32),
            V((NL, D, 128), F32),
            V((NL, D, 128), F32),
            V((NTAB, 8, D), F32),
            V((256, D), U32),
            V((S // 4, 9 * D), U32),
            V((NL, S, 128), F32),
            V((S, D), F32),
            V((7, 320, 256), F32),
            V((D, 128), F32),
            V((D, 128), F32),
            V((NL * 80, 128), U32),
            V((7 * 128, 256), U32),
            V((64, 512), U32),
            V((320, 128), U32),
            V((8, D), F32),
            V((2, 8, D), F32),
            V((S, D), F32),
            V((7 * 160, 256), U32),
            V((320, 128), U32),
            V((7 * 128, 256), U32),
            V((256, 128), U32),
            V((64, D), U32),
            V((5 * 128, 256), U32),
            V((128, 2048), U32),
            V((7 * 320, 256), U32),
            V((S, 128), F32),
            V((D // 2, D), U32),
            V((D,), BF16), V((D,), BF16), V((D,), BF16), V((D,), BF16),
            pltpu.SemaphoreType.DMA((11,)),
            pltpu.SemaphoreType.DMA((1,)),
        ],
        compiler_params=pltpu.CompilerParams(vmem_limit_bytes=110 * 1024 * 1024,
                                             disable_bounds_checks=True,
                                             disable_semaphore_checks=True),
    )(A_x, A_wqkv, A_wo, B_x, B_Lambda_re, B_Lambda_im, B_B_re, B_B_im,
      B_C_re, B_C_im, B_log_dt, B_Dskip)
```

```python
import jax
import jax.numpy as jnp
from jax import lax
from jax.experimental import pallas as pl
from jax.experimental.pallas import tpu as pltpu

S = 2048
D = 640
NL = 5
H = 32
DH = 20
TB = 256
SEGS = (20, 12)
BASES = (0, 8 * SEGS[0])
NB = 32

F32 = jnp.float32
BF16 = jnp.bfloat16
U32 = jnp.uint32
NT = (((1,), (1,)), ((), ()))

T_LR, T_LI, T_D, T_CR, T_CI, T_NCI = 0, 1, 2, 3, 4, 5


def _tab_idx(sub, k, part):
    return 6 + sub * 8 + k * 2 + part


NTAB = 6 + 16

ORD = (2, 3, 1, 0, 5, 4, 6)
ORDK = (2, 4, 3, 0, 6, 1, 5)
ORDG = (2, 3, 4, 1, 0, 5, 6)
ORDY0 = (1, 4, 0, 3, 6, 2, 5)

KTOP = ((0, 128), (256, 384), (512, 576))
KBOT = ((128, 256), (384, 512), (576, 640))
KVR = ((0, 144), (112, 272), (240, 400), (368, 528), (496, 640))


def _cmul(ar, ai, br, bi):
    return ar * br - ai * bi, ar * bi + ai * br


def _phi(t):
    return jnp.where(t > 0, t + 1.0, jnp.exp(t)) + 1e-6


def _pk(x):
    return pltpu.bitcast(x.astype(BF16), U32)


def _up(x):
    return pltpu.bitcast(x, BF16)


def _sums_a(a11, a12, a21, a22):
    return [a11 + a22, a21 + a22, a11, a22, a11 + a12, a21 - a11, a12 - a22]


def _op_b(i, g):
    return [lambda: g(0, 0) + g(1, 1), lambda: g(0, 0), lambda: g(0, 1) - g(1, 1),
            lambda: g(1, 0) - g(0, 0), lambda: g(1, 1), lambda: g(0, 0) + g(0, 1),
            lambda: g(1, 0) + g(1, 1)][i]()


def _combine(m):
    return (m[0] + m[3] - m[4] + m[6], m[2] + m[4], m[1] + m[3], m[0] - m[1] + m[2] + m[5])


def _lt(x, lt):
    return x[:, lt * 128:(lt + 1) * 128]


def _dot_nt(a, b):
    return lax.dot_general(a, b, NT, preferred_element_type=F32)


def _dot(a, b):
    return jnp.dot(a, b, preferred_element_type=F32)


def _kernel(xa_hbm, wqkv_hbm, wo_hbm, xb_hbm, lre_hbm, lim_hbm, bre_hbm, bim_hbm,
            cre_hbm, cim_hbm, ldt_hbm, dsk_hbm,
            out_hbm,
            xa, xb, xw, wq, wk, wv, wo, bcat, cre, cim, cS, cR, slab, slab2, tab,
            xp, hb, ys, oa, gM, gR, zacc, kvs, mS, mKR, mNR, zrow, carry_ref, pqs,
            wkS, wkR, wqS, wqKR, wqNR, xS, xpS, bS, rrs, gb,
            v_lre, v_lim, v_ldt, v_dsk, sem_in, sem_out):
    groups = {}

    def cp(g, src, dst):
        c = pltpu.make_async_copy(src, dst, sem_in.at[g])
        c.start()
        groups.setdefault(g, []).append(c)

    def cp_rows(g, src, dst, r0, n, d0=None):
        d0 = r0 if d0 is None else d0
        cp(g, src.at[pl.ds(r0, n), :], dst.at[pl.ds(d0, n), :])

    def wait(g):
        for c in groups[g]:
            c.wait()

    xb_h = xb_hbm.at[0]
    xa_h = xa_hbm.at[0]

    def it_copies(i):
        a0 = i * 512
        t0 = 1024 + i * TB
        if not isinstance(i, int):
            a0 = pl.multiple_of(a0, 512)
            t0 = pl.multiple_of(t0, TB)
        return (pltpu.make_async_copy(xa_h.at[pl.ds(a0, 512), :], xa.at[pl.ds(a0, 512), :],
                                      sem_in.at[7 + i]),
                pltpu.make_async_copy(xb_h.at[pl.ds(t0, TB), :], xb.at[pl.ds(t0, TB), :],
                                      sem_in.at[7 + i]))

    cp(6, lre_hbm, v_lre)
    cp(6, lim_hbm, v_lim)
    cp(6, ldt_hbm, v_ldt)
    cp(6, dsk_hbm, v_dsk)
    cp_rows(0, xb_h, xb, 0, 512)
    cp_rows(1, bre_hbm, bcat, 0, 256)
    cp_rows(2, bim_hbm, bcat, 0, 256, D)
    cp_rows(2, bre_hbm, bcat, 256, 256)
    cp_rows(3, bim_hbm, bcat, 256, 384, D + 256)
    cp_rows(3, bre_hbm, bcat, 512, 128)
    cp_rows(3, xb_h, xb, 512, 512)
    cp(4, wqkv_hbm.at[:, pl.ds(D, D)], wk)
    cp(4, cre_hbm, cre)
    cp(4, cim_hbm, cim)
    cp(4, wqkv_hbm.at[:, pl.ds(0, D)], wq)
    for i in range(4):
        for c in it_copies(i):
            c.start()
    cp(5, wqkv_hbm.at[:, pl.ds(2 * D, D)], wv)
    cp(5, wo_hbm, wo)

    def out_b(t0, lt):
        return pltpu.make_async_copy(
            ys.at[lt, pl.ds(t0, TB), :],
            out_hbm.at[0, pl.ds(t0, TB), pl.ds(D + lt * 128, 128)], sem_out.at[0])

    def out_a(a0, n):
        return pltpu.make_async_copy(
            oa.at[pl.ds(a0, n), :], out_hbm.at[0, pl.ds(a0, n), pl.ds(0, D)], sem_out.at[0])

    frac = {}

    def chunk(c):
        t0 = pl.multiple_of(c * TB, TB)
        frac[id(t0)] = (pl.multiple_of(c * (TB // 2), TB // 2), pl.multiple_of(c * (TB // 4), TB // 4))
        return t0

    def half(t0):
        return t0 // 2 if isinstance(t0, int) else frac[id(t0)][0]

    def quarter(t0):
        return t0 // 4 if isinstance(t0, int) else frac[id(t0)][1]

    def b_stage(r0):
        for lt in range(NL):
            xw[pl.ds(lt * (S // 2) + half(r0), TB // 2), :] = pltpu.bitcast(
                xb[pl.ds(r0, TB), lt * 128:(lt + 1) * 128], U32)

    def b_ld2(r0, g, lt):
        si = 0 if g < SEGS[0] else 1
        j = g - (0 if si == 0 else SEGS[0])
        w = xw[pl.ds(lt * (S // 2) + half(r0) + (BASES[si] + j) // 2, 8, stride=SEGS[si] // 2), :]
        lo = pltpu.bitcast(w << 16, F32)
        hi = pltpu.bitcast(w & jnp.uint32(0xFFFF0000), F32)
        return jnp.concatenate([lo, hi], axis=0)

    def b_prep(r0):
        for g in range(0, 32, 2):
            for lt in range(NL):
                xp[r0 // 2 + 4 * g:r0 // 2 + 4 * g + 8, lt * 128:(lt + 1) * 128] = _pk(b_ld2(r0, g, lt))

    def b_prep_s(tops, bots):
        for k in range(len(tops)):
            tl = [b_ld2(*tops[k], lt) for lt in range(NL)]
            bl = [b_ld2(*bots[k], lt) for lt in range(NL)]
            for c in range(2):
                for i, v in enumerate(_sums_a(tl[c], tl[2 + c], bl[c], bl[2 + c])):
                    xpS[8 * k:8 * k + 8, i * 256 + c * 128:i * 256 + (c + 1) * 128] = _pk(v)
            xpS[8 * k:8 * k + 8, 1792:1920] = _pk(tl[4])
            xpS[8 * k:8 * k + 8, 1920:2048] = _pk(bl[4])
        return 16 * len(tops)

    def bs_op(p, i):
        if i in (1, 4):
            return
        for r in range(p * 128, (p + 1) * 128, 32):
            for c in range(2):
                g = lambda kh, nh: bcat[nh * D + r:nh * D + r + 32,
                                        (2 * kh + c) * 128:(2 * kh + c + 1) * 128].astype(F32)
                bS[i * 320 + r // 2:i * 320 + r // 2 + 16, c * 128:(c + 1) * 128] = _pk(_op_b(i, g))

    def bu_prod(hn, p, i):
        if i == 1:
            w = bcat[p * 128:(p + 1) * 128, 0:256]
        elif i == 4:
            w = bcat[D + p * 128:D + (p + 1) * 128, 256:512]
        else:
            w = _up(bS[i * 320 + p * 64:i * 320 + (p + 1) * 64, :])
        return _dot_nt(_up(xpS[0:hn // 2, i * 256:(i + 1) * 256]), w)

    def bu_rem(hn, p):
        xr = jnp.concatenate([_up(xpS[0:hn // 2, 1792:1920]), _up(xpS[0:hn // 2, 1920:2048])], axis=0)
        w = jnp.concatenate([bcat[p * 128:(p + 1) * 128, 512:640],
                             bcat[D + p * 128:D + (p + 1) * 128, 512:640]], axis=0)
        return _dot_nt(xr, w)

    def bu_fin(m, rem):
        c11, c12, c21, c22 = _combine(m)
        return (jnp.concatenate([c11, c21], axis=0) + rem[:, 0:128],
                jnp.concatenate([c12, c22], axis=0) + rem[:, 128:256])

    def bu_plain(x, tiles):
        w = jnp.concatenate([bcat[t * 128:(t + 1) * 128, :] for t in tiles], axis=0)
        r = _dot_nt(x, w)
        return {t: _lt(r, i) for i, t in enumerate(tiles)}

    carry = {}

    def b_scan(items):
        sub8 = lax.broadcasted_iota(jnp.int32, (8, 128), 0)
        chains = []
        for bu, t0, lt in items:
            for c in range(bu[0].shape[0] // TB):
                for si in range(2):
                    chains.append((bu, c * TB + BASES[si], si, lt, t0))
        lam = {lt: (tab[T_LR, :, lt * 128:(lt + 1) * 128], tab[T_LI, :, lt * 128:(lt + 1) * 128])
               for _, _, lt in items}
        tb = lambda si, k, lt: (tab[_tab_idx(si, k, 0), :, lt * 128:(lt + 1) * 128],
                                tab[_tab_idx(si, k, 1), :, lt * 128:(lt + 1) * 128])
        ld = lambda bu, r: (bu[0][r:r + 8, :], bu[1][r:r + 8, :])

        def step(h, a, b):
            return (a[0] * h[0] - a[1] * h[1] + b[0], a[0] * h[1] + a[1] * h[0] + b[1])

        st = [ld(bu, o) for bu, o, si, lt, t0 in chains]
        for j in range(1, max(SEGS)):
            for ix, (bu, o, si, lt, t0) in enumerate(chains):
                if j < SEGS[si]:
                    st[ix] = step(st[ix], lam[lt], ld(bu, o + 8 * j))
        for k in range(3):
            for ix, (bu, o, si, lt, t0) in enumerate(chains):
                e = st[ix]
                sh = (pltpu.roll(e[0], 1 << k, 0), pltpu.roll(e[1], 1 << k, 0))
                st[ix] = step(sh, tb(si, k, lt), e)
        for ix, (bu, o, si, lt, t0) in enumerate(chains):
            rl = tuple(jnp.where(sub8 == 0, 0.0, pltpu.roll(v, 1, 0)) for v in st[ix])
            prev = carry.get(lt)
            h = rl if prev is None else step(prev, tb(si, 3, lt), rl)
            for j in range(0, SEGS[si], 4):
                r = o + 8 * j
                h1 = step(h, lam[lt], ld(bu, r))
                h2 = step(h1, lam[lt], ld(bu, r + 8))
                h3 = step(h2, lam[lt], ld(bu, r + 16))
                h = step(h3, lam[lt], ld(bu, r + 24))
                cat = lambda a, b: jnp.concatenate([a, b], axis=0)
                a11, a12 = cat(h1[0], h2[0]), cat(h1[1], h2[1])
                a21, a22 = cat(h3[0], h[0]), cat(h3[1], h[1])
                sm = _sums_a(a11, a12, a21, a22)
                rows = pl.ds(quarter(t0) + r // 4, 8)
                for k, v in enumerate([a11, a12, a21, a22, sm[0], sm[1], sm[4], sm[5], sm[6]]):
                    hb[rows, k * D + lt * 128:k * D + (lt + 1) * 128] = _pk(v)
            carry[lt] = tuple(jnp.broadcast_to(v[7:8, :], (8, 128)) for v in h)

    def carry_save():
        for lt in range(NL):
            carry_ref[0, :, lt * 128:(lt + 1) * 128] = carry[lt][0]
            carry_ref[1, :, lt * 128:(lt + 1) * 128] = carry[lt][1]

    def carry_load():
        for lt in range(NL):
            carry[lt] = (carry_ref[0, :, lt * 128:(lt + 1) * 128],
                         carry_ref[1, :, lt * 128:(lt + 1) * 128])

    def y_store(t0, ytop, ybot, lt):
        dv = tab[T_D, :, lt * 128:(lt + 1) * 128]
        for base, n in zip(BASES, SEGS):
            for j in range(0, n, 2):
                xv = b_ld2(t0, base // 8 + j, lt)
                r = (base + 8 * (j - j % 4)) // 2
                y = ytop if j % 4 < 2 else ybot
                for e in range(2):
                    idx = pl.ds(t0 + base + j + e, 8, stride=n)
                    ys[lt, idx, :] = y[r + 8 * e:r + 8 * e + 8, :] + xv[8 * e:8 * e + 8] * dv
        out_b(t0, lt).start()

    hidx = {0: 4, 1: 5, 2: 0, 3: 3, 4: 6, 5: 7, 6: 8}

    def y_main(t0, order=ORD):
        rows = pl.ds(quarter(t0), TB // 4)
        m = [None] * 7
        for i in order:
            m[i] = _dot_nt(_up(hb[rows, hidx[i] * D:(hidx[i] + 1) * D]),
                           _up(cS[i * 128:(i + 1) * 128, :]))
        c11, c12, c21, c22 = _combine(m)
        for c in range(2):
            y_store(t0, _lt(c12, c), _lt(c22, c), 2 + c)
        for c in range(2):
            y_store(t0, _lt(c11, c), _lt(c21, c), c)

    def y_rem(t0):
        rows = pl.ds(quarter(t0), TB // 4)
        h = jnp.concatenate([_up(hb[rows, 0:2 * D]), _up(hb[rows, 2 * D:4 * D])], axis=0)
        y = _dot_nt(h, _up(cR[...]))
        y_store(t0, y[0:128], y[128:256], 4)

    def tables():
        lre = v_lre[...].astype(F32).reshape(1, D)
        lim = v_lim[...].astype(F32).reshape(1, D)
        dt = jnp.exp(v_ldt[...].astype(F32).reshape(1, D)).astype(BF16).astype(F32)
        dsk = v_dsk[...].astype(F32).reshape(1, D)
        mag = jnp.exp(dt * lre)
        ang = dt * lim
        lbr = mag * jnp.cos(ang)
        lbi = mag * jnp.sin(ang)
        sc = jnp.maximum(jnp.abs(lre), jnp.abs(lim))
        a_ = lre / sc
        b_ = lim / sc
        dn = (a_ * a_ + b_ * b_) * sc
        nr = lbr - 1.0
        cr = (nr * a_ + lbi * b_) / dn
        ci = (lbi * a_ - nr * b_) / dn
        bc = lambda v: jnp.broadcast_to(v, (8, D))
        sub = lax.broadcasted_iota(jnp.int32, (8, D), 0)
        tab[T_LR] = bc(lbr)
        tab[T_LI] = bc(lbi)
        tab[T_D] = bc(dsk)
        tab[T_CR] = bc(2.0 * cr)
        tab[T_CI] = bc(2.0 * ci)
        tab[T_NCI] = bc(-2.0 * ci)
        pw = [(lbr, lbi)]
        for _ in range(4):
            pw.append(_cmul(*pw[-1], *pw[-1]))
        for si, n in enumerate(SEGS):
            acc = None
            for b in range(5):
                if (n >> b) & 1:
                    acc = pw[b] if acc is None else _cmul(*acc, *pw[b])
            w = (jnp.ones((8, D), F32), jnp.zeros((8, D), F32))
            for k in range(3):
                a8 = (bc(acc[0]), bc(acc[1]))
                tab[_tab_idx(si, k, 0)] = jnp.where(sub >= (1 << k), a8[0], 0.0)
                tab[_tab_idx(si, k, 1)] = jnp.where(sub >= (1 << k), a8[1], 0.0)
                wm = _cmul(*w, *a8)
                bit = ((sub >> k) & 1) == 1
                w = (jnp.where(bit, wm[0], w[0]), jnp.where(bit, wm[1], w[1]))
                if k < 2:
                    acc = _cmul(*acc, *acc)
            tab[_tab_idx(si, 3, 0)] = w[0]
            tab[_tab_idx(si, 3, 1)] = w[1]

    def c_prep():
        def pq(r, lt, which):
            cs = slice(lt * 128, (lt + 1) * 128)
            c_r = cre[r:r + 16, cs].astype(F32)
            c_i = cim[r:r + 16, cs].astype(F32)
            if which == 0:
                return c_r * tab[T_CR, 0:1, cs] - c_i * tab[T_CI, 0:1, cs]
            return c_r * tab[T_NCI, 0:1, cs] - c_i * tab[T_CR, 0:1, cs]

        def put(i, r, lt, v):
            cS[i * 128 + r // 2:i * 128 + r // 2 + 8, lt * 128:(lt + 1) * 128] = _pk(v)

        p1, q2 = {}, {}
        pos = [(r, lt) for r in range(0, 256, 16) for lt in range(NL)]
        for r, lt in pos:
            p1[r, lt] = pq(r, lt, 0)
            put(1, r, lt, p1[r, lt])
        for r, lt in pos:
            q2[r, lt] = pq(256 + r, lt, 1)
            put(4, r, lt, q2[r, lt])
            put(0, r, lt, p1[r, lt] + q2[r, lt])
        for r, lt in pos:
            q1 = pq(r, lt, 1)
            put(3, r, lt, q1 - p1[r, lt])
            put(6, r, lt, q1 + q2[r, lt])
        for r, lt in pos:
            p2 = pq(256 + r, lt, 0)
            put(2, r, lt, p2 - q2[r, lt])
            put(5, r, lt, p1[r, lt] + p2)
        for which in range(2):
            for r in range(0, 128, 16):
                for lt in range(NL):
                    cR[r // 2:r // 2 + 8, which * D + lt * 128:which * D + (lt + 1) * 128] = _pk(
                        pq(512 + r, lt, which))

    def wk_prep():
        blk = lambda kt, ft: wk[kt * 128:(kt + 1) * 128, ft * 128:(ft + 1) * 128].astype(F32)
        rnd = lambda v: v.astype(BF16).astype(F32)
        for i in ORDK:
            for fp in range(2):
                for c in range(2):
                    v = _op_b(i, lambda kh, nh: blk(2 * kh + c, 2 * fp + nh))
                    wkS[i * 160 + fp * 64:i * 160 + (fp + 1) * 64, c * 128:(c + 1) * 128] = _pk(rnd(v).T)
        for c in range(2):
            t = [blk(c, 4).T, blk(2 + c, 4).T]
            for i in range(7):
                v = _op_b(i, lambda kh, nh: t[kh][64 * nh:64 * (nh + 1)])
                wkS[i * 160 + 128:i * 160 + 160, c * 128:(c + 1) * 128] = _pk(v)
        pos = 0
        tr = [blk(4, ft).T for ft in range(NL)]
        for lo, hi in KTOP + KBOT:
            wkR[pos // 2:(pos + hi - lo) // 2, :] = _pk(tr[lo // 128][lo % 128:lo % 128 + hi - lo])
            pos += hi - lo

    def wq_transpose():
        for lt in range(NL):
            slab2[lt] = wq[lt * 128:(lt + 1) * 128, :].astype(F32).T

    def wq_ops():
        g = lambda d, lt: slab2[lt, pl.ds(d, H, stride=DH), :]
        for i in ORD:
            for d in range(8):
                for c in range(2):
                    v = _op_b(i, lambda kh, nh: g(d + 8 * nh, 2 * kh + c))
                    wqS[i * 128 + d * 16:i * 128 + (d + 1) * 16, c * 128:(c + 1) * 128] = _pk(v)
        for d in range(16):
            wqKR[d * 16:(d + 1) * 16, :] = _pk(g(d, 4))
        for d in range(16, 20):
            for lt in range(NL):
                wqNR[(d - 16) * 16:(d - 15) * 16, lt * 128:(lt + 1) * 128] = _pk(g(d, lt))

    xidx = {0: 0, 1: 1, 4: 2, 5: 3, 6: 4}

    def x_sums(a0):
        for r in range(0, 256, 32):
            for c in range(2):
                g = lambda ro, co: xa[pl.ds(a0 + ro + r, 32),
                                      (co + c) * 128:(co + c + 1) * 128].astype(F32)
                sm = _sums_a(g(0, 0), g(0, 2), g(256, 0), g(256, 2))
                for i, k in xidx.items():
                    xS[k * 128 + r // 2:k * 128 + r // 2 + 16, c * 128:(c + 1) * 128] = _pk(sm[i])

    def x_op(a0, i):
        if i == 2:
            return xa[pl.ds(a0, 256), 0:256]
        if i == 3:
            return xa[pl.ds(a0 + 256, 256), 256:512]
        return _up(xS[xidx[i] * 128:(xidx[i] + 1) * 128, :])

    def a_k(a0):
        rem = _dot_nt(_up(wkR[...]), xa[pl.ds(a0, 512), 512:640])
        m = [None] * 7
        for i in ORDK:
            m[i] = _dot_nt(_up(wkS[i * 160:(i + 1) * 160, :]), x_op(a0, i))
        c11, c12, c21, c22 = _combine(m)
        a11 = _phi(c11 + rem[0:320, 0:256])
        a12 = _phi(c21 + rem[0:320, 256:512])
        a21 = _phi(c12 + rem[320:640, 0:256])
        a22 = _phi(c22 + rem[320:640, 256:512])
        zt = (_lt(a11, 0) + _lt(a11, 1)) + (_lt(a12, 0) + _lt(a12, 1))
        zb = (_lt(a21, 0) + _lt(a21, 1)) + (_lt(a22, 0) + _lt(a22, 1))
        for zz, rngs in ((zt, KTOP), (zb, KBOT)):
            pos = 0
            for lo, hi in rngs:
                zacc[lo:hi, :] += zz[pos:pos + hi - lo]
                pos += hi - lo
        ops = [v.astype(BF16) for v in _sums_a(a11, a12, a21, a22)]
        full = jnp.concatenate([jnp.concatenate([ops[2], a12.astype(BF16)], axis=1),
                                jnp.concatenate([a21.astype(BF16), ops[3]], axis=1)], axis=0)
        return ops, full

    gmap = {0: 0, 1: 2, 2: 6, 3: 5, 4: 3, 5: 4, 6: 1}

    def a_q_nrem(a0):
        pqs[pl.ds(a0, 512), 512:640] = _phi(_dot_nt(xa[pl.ds(a0, 512), :], _up(wqNR[...])))

    def a_q(a0):
        rem = _dot_nt(xa[pl.ds(a0, 512), 512:640], _up(wqKR[...]))
        m = [None] * 7
        for i in ORDK:
            m[i] = _dot_nt(x_op(a0, i), _up(wqS[i * 128:(i + 1) * 128, :]))
        c11, c12, c21, c22 = _combine(m)
        pqs[pl.ds(a0, 256), 0:256] = _phi(c11 + rem[0:256, 0:256])
        pqs[pl.ds(a0, 256), 256:512] = _phi(c12 + rem[0:256, 256:512])
        pqs[pl.ds(a0 + 256, 256), 0:256] = _phi(c21 + rem[256:512, 0:256])
        pqs[pl.ds(a0 + 256, 256), 256:512] = _phi(c22 + rem[256:512, 256:512])

    def a_z():
        for lt in range(NL):
            zp = jnp.concatenate(
                [zacc[pl.ds(d, H, stride=DH), :] for d in range(4 * lt, 4 * lt + 4)], axis=0)
            zrow[:, lt * 128:(lt + 1) * 128] = jnp.broadcast_to(
                jnp.sum(zp.T, axis=0, keepdims=True), (8, 128))

    def g_pack(gm, gr):
        c11, c12, c21, c22 = _combine(gm)
        for top, (cl, cr_), rngs in ((0, (c11, c12), KTOP), (320, (c21, c22), KBOT)):
            pos = 0
            for lo, hi in rngs:
                gb[lo // 2:hi // 2, 0:256] = _pk(cl[pos:pos + hi - lo])
                gb[lo // 2:hi // 2, 256:512] = _pk(cr_[pos:pos + hi - lo])
                gb[lo // 2:hi // 2, 512:640] = _pk(gr[top + pos:top + pos + hi - lo])
                pos += hi - lo

    def a_kv():
        for j, (lo, hi) in enumerate(KVR):
            kv = _dot(_up(gb[lo // 2:hi // 2, :]), wv[:, j * 128:(j + 1) * 128])
            rh = (lax.broadcasted_iota(jnp.int32, kv.shape, 0) + lo) // DH
            ch = (lax.broadcasted_iota(jnp.int32, kv.shape, 1) + j * 128) // DH
            kvs[j * 80:j * 80 + (hi - lo) // 2, :] = _pk(jnp.where(rh == ch, kv, 0.0))

    def a_m():
        parts = [_dot(_up(kvs[j * 80:j * 80 + (hi - lo) // 2, :]), wo[j * 128:(j + 1) * 128, :])
                 for j, (lo, hi) in enumerate(KVR)]
        pieces = []
        pos = 0
        for j, (lo, hi) in enumerate(KVR):
            nxt = KVR[j + 1][0] if j + 1 < len(KVR) else hi
            pieces.append(parts[j][pos - lo:nxt - lo])
            if j + 1 < len(KVR):
                pieces.append(parts[j][nxt - lo:hi - lo] + parts[j + 1][0:hi - nxt])
                pos = hi
        m = jnp.concatenate(pieces, axis=0)
        for lt in range(NL):
            slab[lt] = _lt(m, lt)
        g = lambda d, lt: slab[lt, pl.ds(d, H, stride=DH), :]
        for i in ORD:
            for d in range(8):
                for c in range(2):
                    v = _op_b(i, lambda kh, nh: g(d + 8 * kh, 2 * nh + c))
                    mS[i * 128 + d * 16:i * 128 + (d + 1) * 16, c * 128:(c + 1) * 128] = _pk(v)
        for d in range(16, 20):
            for lt in range(4):
                mKR[(d - 16) * 16:(d - 15) * 16, lt * 128:(lt + 1) * 128] = _pk(g(d, lt))
        for d in range(DH):
            mNR[d * 16:(d + 1) * 16, :] = _pk(g(d, 4))

    def a_o(a0, n):
        hn = n // 2
        for r in range(a0, a0 + n, NB):
            t = pqs[r:r + NB, 0:128] * zrow[0:1, 0:128]
            for lt in range(1, NL):
                t = t + pqs[r:r + NB, lt * 128:(lt + 1) * 128] * zrow[0:1, lt * 128:(lt + 1) * 128]
            t = t + pltpu.roll(t, 64, 1)
            t = t + pltpu.roll(t, 32, 1)
            rrs[r:r + NB, :] = 1.0 / (t + 1e-6)

        def norm_rows(r):
            pq = pqs[r:r + NB, :]
            rr = rrs[r:r + NB, :]
            return jnp.concatenate([_lt(pq, lt) * rr for lt in range(NL)], axis=1)

        tops, bots, sums = [], [], [[] for _ in range(7)]
        for r in range(0, hn, NB):
            tp = norm_rows(a0 + r)
            bt = norm_rows(a0 + hn + r)
            sm = _sums_a(tp[:, 0:256], tp[:, 256:512], bt[:, 0:256], bt[:, 256:512])
            tops.append(tp.astype(BF16))
            bots.append(bt.astype(BF16))
            for i in (0, 1, 4, 5, 6):
                sums[i].append(sm[i].astype(BF16))
        full = jnp.concatenate(tops + bots, axis=0)
        ops = [None] * 7
        for i in (0, 1, 4, 5, 6):
            ops[i] = jnp.concatenate(sums[i], axis=0)
        ops[2] = full[0:hn, 0:256]
        ops[3] = full[hn:n, 256:512]
        oa[a0:a0 + n, 512:640] = _dot(full, _up(mNR[...]))
        rem = _dot(full[:, 512:640], _up(mKR[...]))
        m = [None] * 7
        for i in ORD:
            m[i] = _dot(ops[i], _up(mS[i * 128:(i + 1) * 128, :]))
        c11, c12, c21, c22 = _combine(m)
        oa[a0:a0 + hn, 0:256] = c11 + rem[0:hn, 0:256]
        oa[a0:a0 + hn, 256:512] = c12 + rem[0:hn, 256:512]
        oa[a0 + hn:a0 + n, 0:256] = c21 + rem[hn:n, 0:256]
        oa[a0 + hn:a0 + n, 256:512] = c22 + rem[hn:n, 256:512]
        out_a(a0, n).start()

    gM[...] = jnp.zeros(gM.shape, F32)
    gR[...] = jnp.zeros(gR.shape, F32)
    zacc[...] = jnp.zeros(zacc.shape, F32)
    wait(6)
    tables()
    wait(0)
    b_stage(0)
    b_stage(256)
    b_prep(0)
    b_prep(256)

    u = {}

    def sc(ps):
        b_scan([((u.pop(p), u.pop(p + 5)), 0, p) for p in ps])

    wait(1)
    ra = bu_plain(_up(xp[0:128]), [0, 1])
    rb = bu_plain(_up(xp[128:256]), [0, 1])
    u.update({t: jnp.concatenate([ra[t], rb[t]], axis=0) for t in (0, 1)})
    wait(2)
    u.update(bu_plain(_up(xp[...]), [5, 6]))
    sc([0, 1])
    u.update(bu_plain(_up(xp[...]), [2, 3]))
    wait(3)
    u.update(bu_plain(_up(xp[...]), [7, 8]))
    sc([2, 3])
    u.update(bu_plain(_up(xp[...]), [4, 9]))
    sc([4])

    b_stage(512)
    b_stage(768)
    hn = b_prep_s([(512, g) for g in range(0, 32, 2)], [(768, g) for g in range(0, 32, 2)])
    mt = {}

    def rem1(p):
        mt[p] = ([None] * 7, bu_rem(hn, p))

    def prod1(p, k0, k1):
        for k in range(k0, k1):
            bs_op(p, ORD[k])
            mt[p][0][ORD[k]] = bu_prod(hn, p, ORD[k])
        if k1 == 7:
            b_scan([(bu_fin(*mt[p]), 512, p)])

    rem1(0)
    rem1(1)
    rem1(2)
    prod1(0, 0, 7)
    prod1(1, 0, 7)
    prod1(2, 0, 7)
    rem1(3)
    prod1(3, 0, 3)
    wait(4)
    c_prep()
    prod1(3, 3, 5)
    rem1(4)
    y_main(0, ORDY0)
    prod1(3, 5, 7)
    prod1(4, 0, 7)
    y_main(TB)
    y_rem(0)
    y_rem(TB)
    carry_save()
    wk_prep()
    wq_transpose()

    def main(i, c):
        for cc in it_copies(i):
            cc.wait()
        a0 = pl.multiple_of(i * 512, 512)
        tb0 = chunk(i + 4)
        ty = chunk(i + 2)
        b_stage(tb0)
        x_sums(a0)
        wq_ops()
        y_rem(ty)
        ops, full = a_k(a0)
        a_q_nrem(a0)
        h2 = b_prep_s([(tb0, g) for g in range(0, 16, 2)], [(tb0, g) for g in range(16, 32, 2)])
        carry_load()
        for p in range(NL):
            rem = bu_rem(h2, p)
            m = [None] * 7
            for k in ORD:
                m[k] = bu_prod(h2, p, k)
            b_scan([(bu_fin(m, rem), tb0, p)])
        carry_save()
        gm = [None] * 7
        for k in ORDG:
            gm[k] = gM[k] + _dot(ops[k], x_op(a0, gmap[k]))
            gM[k] = gm[k]
        a_q(a0)
        y_main(ty)
        gr = gR[...] + _dot(full, xa[pl.ds(a0, 512), 512:640])
        gR[...] = gr
        g_pack(gm, gr)
        a_z()
        return c

    lax.fori_loop(0, 4, main, 0)

    wait(5)
    a_kv()
    y_main(6 * TB)
    a_m()
    y_rem(6 * TB)
    for i in range(8):
        a_o(i * 256, 256)
    y_main(7 * TB)
    y_rem(7 * TB)

    for c in range(8):
        for lt in range(NL):
            out_b(c * TB, lt).wait()
    for i in range(8):
        out_a(i * 256, 256).wait()


def _compiler_params():
    base = dict(vmem_limit_bytes=110 * 1024 * 1024)
    for extra in (dict(disable_bounds_checks=True, disable_semaphore_checks=True),
                  dict(disable_bounds_checks=True), dict()):
        try:
            return pltpu.CompilerParams(**base, **extra)
        except TypeError:
            continue
    return None


@jax.jit
def pallas_concat_heads__linear_attn_block__ssm_conv_s5__prompt_kernel(
    A_x: jax.Array,
    A_wqkv: jax.Array,
    A_wo: jax.Array,
    B_x: jax.Array,
    B_Lambda_re: jax.Array,
    B_Lambda_im: jax.Array,
    B_B_re: jax.Array,
    B_B_im: jax.Array,
    B_C_re: jax.Array,
    B_C_im: jax.Array,
    B_log_dt: jax.Array,
    B_Dskip: jax.Array,
):
    any_spec = pl.BlockSpec(memory_space=pl.ANY)
    V = pltpu.VMEM
    return pl.pallas_call(
        _kernel,
        out_shape=jax.ShapeDtypeStruct((1, S, 2 * D), F32),
        in_specs=[any_spec] * 12,
        out_specs=any_spec,
        scratch_shapes=[
            V((S, D), BF16),
            V((S, D), BF16),
            V((NL * (S // 2), 128), U32),
            V((D, D), BF16),
            V((D, D), BF16),
            V((D, D), BF16),
            V((D, D), BF16),
            V((2 * D, D), BF16),
            V((D, D), BF16),
            V((D, D), BF16),
            V((7 * 128, D), U32),
            V((64, 2 * D), U32),
            V((NL, D, 128), F32),
            V((NL, D, 128), F32),
            V((NTAB, 8, D), F32),
            V((256, D), U32),
            V((S // 4, 9 * D), U32),
            V((NL, S, 128), F32),
            V((S, D), F32),
            V((7, 320, 256), F32),
            V((D, 128), F32),
            V((D, 128), F32),
            V((NL * 80, 128), U32),
            V((7 * 128, 256), U32),
            V((64, 512), U32),
            V((320, 128), U32),
            V((8, D), F32),
            V((2, 8, D), F32),
            V((S, D), F32),
            V((7 * 160, 256), U32),
            V((320, 128), U32),
            V((7 * 128, 256), U32),
            V((256, 128), U32),
            V((64, D), U32),
            V((5 * 128, 256), U32),
            V((128, 2048), U32),
            V((7 * 320, 256), U32),
            V((S, 128), F32),
            V((D // 2, D), U32),
            V((D,), BF16), V((D,), BF16), V((D,), BF16), V((D,), BF16),
            pltpu.SemaphoreType.DMA((11,)),
            pltpu.SemaphoreType.DMA((1,)),
        ],
        compiler_params=_compiler_params(),
    )(A_x, A_wqkv, A_wo, B_x, B_Lambda_re, B_Lambda_im, B_B_re, B_B_im,
      B_C_re, B_C_im, B_log_dt, B_Dskip)
```

```python
import jax
import jax.numpy as jnp
from jax import lax
from jax.experimental import pallas as pl
from jax.experimental.pallas import tpu as pltpu

S = 2048
D = 640
NL = 5
H = 32
DH = 20
TB = 256
SEGS = (20, 12)
BASES = (0, 8 * SEGS[0])
NB = 32
N0 = 4

F32 = jnp.float32
BF16 = jnp.bfloat16
U32 = jnp.uint32
NT = (((1,), (1,)), ((), ()))

T_LR, T_LI, T_D, T_CR, T_CI, T_NCI = 0, 1, 2, 3, 4, 5


def _tab_idx(sub, k, part):
    return 6 + sub * 8 + k * 2 + part


NTAB = 6 + 16

ORD = (2, 3, 1, 0, 5, 4, 6)
ORDK = (2, 4, 3, 0, 6, 1, 5)
ORDG = (2, 3, 4, 1, 0, 5, 6)
ORDY0 = (1, 4, 0, 3, 6, 2, 5)

KTOP = ((0, 128), (256, 384), (512, 576))
KBOT = ((128, 256), (384, 512), (576, 640))
KVR = ((0, 144), (112, 272), (240, 400), (368, 528), (496, 640))


def _cmul(ar, ai, br, bi):
    return ar * br - ai * bi, ar * bi + ai * br


def _phi(t):
    return jnp.where(t > 0, t + 1.0, jnp.exp(t)) + 1e-6


def _pk(x):
    return pltpu.bitcast(x.astype(BF16), U32)


def _up(x):
    return pltpu.bitcast(x, BF16)


def _sums_a(a11, a12, a21, a22):
    return [a11 + a22, a21 + a22, a11, a22, a11 + a12, a21 - a11, a12 - a22]


def _op_b(i, g):
    return [lambda: g(0, 0) + g(1, 1), lambda: g(0, 0), lambda: g(0, 1) - g(1, 1),
            lambda: g(1, 0) - g(0, 0), lambda: g(1, 1), lambda: g(0, 0) + g(0, 1),
            lambda: g(1, 0) + g(1, 1)][i]()


def _combine(m):
    return (m[0] + m[3] - m[4] + m[6], m[2] + m[4], m[1] + m[3], m[0] - m[1] + m[2] + m[5])


def _lt(x, lt):
    return x[:, lt * 128:(lt + 1) * 128]


def _dot_nt(a, b):
    return lax.dot_general(a, b, NT, preferred_element_type=F32)


def _dot(a, b):
    return jnp.dot(a, b, preferred_element_type=F32)


def _kernel(xa_hbm, wqkv_hbm, wo_hbm, xb_hbm, lre_hbm, lim_hbm, bre_hbm, bim_hbm,
            cre_hbm, cim_hbm, ldt_hbm, dsk_hbm,
            out_hbm,
            xa, xb, xw, wq, wk, wv, wo, bcat, cre, cim, cS, cR, slab, slab2, tab,
            xp, hb, ys, oa, gM, gR, zacc, kvs, mS, mKR, mNR, zrow, carry_ref, pqs,
            wkS, wkR, wqS, wqKR, wqNR, xS, xpS, bS, rrs, gb,
            v_lre, v_lim, v_ldt, v_dsk, sem_in, sem_out):
    groups = {}

    def cp(g, src, dst):
        c = pltpu.make_async_copy(src, dst, sem_in.at[g])
        c.start()
        groups.setdefault(g, []).append(c)

    def cp_blk(g, src, dst, r0, n, c0, w, d0=None):
        d0 = r0 if d0 is None else d0
        cp(g, src.at[pl.ds(r0, n), pl.ds(c0, w)], dst.at[pl.ds(d0, n), pl.ds(c0, w)])

    def wait(g):
        for c in groups[g]:
            c.wait()

    xb_h = xb_hbm.at[0]
    xa_h = xa_hbm.at[0]

    def it_copies(i):
        a0 = i * 512
        t0 = 1024 + i * TB
        if not isinstance(i, int):
            a0 = pl.multiple_of(a0, 512)
            t0 = pl.multiple_of(t0, TB)
        return (pltpu.make_async_copy(xa_h.at[pl.ds(a0, 512), :], xa.at[pl.ds(a0, 512), :],
                                      sem_in.at[7 + i]),
                pltpu.make_async_copy(xb_h.at[pl.ds(t0, TB), :], xb.at[pl.ds(t0, TB), :],
                                      sem_in.at[7 + i]))

    cp(6, lre_hbm, v_lre)
    cp(6, lim_hbm, v_lim)
    cp(6, ldt_hbm, v_ldt)
    cp(6, dsk_hbm, v_dsk)
    cp_blk(0, xb_h, xb, 0, 512, 0, 256)
    cp_blk(0, bre_hbm, bcat, 0, N0 * 128, 0, 256)
    cp_blk(1, bre_hbm, bcat, N0 * 128, D - N0 * 128, 0, 256)
    cp_blk(1, bim_hbm, bcat, 0, D, 0, 256, D)
    cp_blk(2, xb_h, xb, 0, 512, 256, 384)
    cp_blk(2, bre_hbm, bcat, 0, 512, 256, 384)
    cp_blk(2, bim_hbm, bcat, 0, 256, 256, 384, D)
    cp_blk(3, bim_hbm, bcat, 256, 384, 256, 384, D + 256)
    cp_blk(3, bre_hbm, bcat, 512, 128, 256, 384)
    cp(3, xb_h.at[pl.ds(512, 512), :], xb.at[pl.ds(512, 512), :])
    cp(4, wqkv_hbm.at[:, pl.ds(D, D)], wk)
    cp(4, cre_hbm, cre)
    cp(4, cim_hbm, cim)
    cp(4, wqkv_hbm.at[:, pl.ds(0, D)], wq)
    for i in range(4):
        for c in it_copies(i):
            c.start()
    cp(5, wqkv_hbm.at[:, pl.ds(2 * D, D)], wv)
    cp(5, wo_hbm, wo)

    def out_b(t0, lt):
        return pltpu.make_async_copy(
            ys.at[lt, pl.ds(t0, TB), :],
            out_hbm.at[0, pl.ds(t0, TB), pl.ds(D + lt * 128, 128)], sem_out.at[0])

    def out_a(a0, n):
        return pltpu.make_async_copy(
            oa.at[pl.ds(a0, n), :], out_hbm.at[0, pl.ds(a0, n), pl.ds(0, D)], sem_out.at[0])

    frac = {}

    def chunk(c):
        t0 = pl.multiple_of(c * TB, TB)
        frac[id(t0)] = (pl.multiple_of(c * (TB // 2), TB // 2), pl.multiple_of(c * (TB // 4), TB // 4))
        return t0

    def half(t0):
        return t0 // 2 if isinstance(t0, int) else frac[id(t0)][0]

    def quarter(t0):
        return t0 // 4 if isinstance(t0, int) else frac[id(t0)][1]

    def b_stage(r0, lts=range(NL)):
        for lt in lts:
            xw[pl.ds(lt * (S // 2) + half(r0), TB // 2), :] = pltpu.bitcast(
                xb[pl.ds(r0, TB), lt * 128:(lt + 1) * 128], U32)

    def b_ld2(r0, g, lt):
        si = 0 if g < SEGS[0] else 1
        j = g - (0 if si == 0 else SEGS[0])
        w = xw[pl.ds(lt * (S // 2) + half(r0) + (BASES[si] + j) // 2, 8, stride=SEGS[si] // 2), :]
        lo = pltpu.bitcast(w << 16, F32)
        hi = pltpu.bitcast(w & jnp.uint32(0xFFFF0000), F32)
        return jnp.concatenate([lo, hi], axis=0)

    def b_prep(r0, lts):
        b_stage(r0, lts)
        for g in range(0, 32, 2):
            for lt in lts:
                xp[r0 // 2 + 4 * g:r0 // 2 + 4 * g + 8, lt * 128:(lt + 1) * 128] = _pk(b_ld2(r0, g, lt))

    def b_prep_s(tops, bots):
        for k in range(len(tops)):
            tl = [b_ld2(*tops[k], lt) for lt in range(NL)]
            bl = [b_ld2(*bots[k], lt) for lt in range(NL)]
            for c in range(2):
                for i, v in enumerate(_sums_a(tl[c], tl[2 + c], bl[c], bl[2 + c])):
                    xpS[8 * k:8 * k + 8, i * 256 + c * 128:i * 256 + (c + 1) * 128] = _pk(v)
            xpS[8 * k:8 * k + 8, 1792:1920] = _pk(tl[4])
            xpS[8 * k:8 * k + 8, 1920:2048] = _pk(bl[4])
        return 16 * len(tops)

    def bs_op(p, i):
        if i in (1, 4):
            return
        for r in range(p * 128, (p + 1) * 128, 32):
            for c in range(2):
                g = lambda kh, nh: bcat[nh * D + r:nh * D + r + 32,
                                        (2 * kh + c) * 128:(2 * kh + c + 1) * 128].astype(F32)
                bS[i * 320 + r // 2:i * 320 + r // 2 + 16, c * 128:(c + 1) * 128] = _pk(_op_b(i, g))

    def bu_prod(hn, p, i):
        if i == 1:
            w = bcat[p * 128:(p + 1) * 128, 0:256]
        elif i == 4:
            w = bcat[D + p * 128:D + (p + 1) * 128, 256:512]
        else:
            w = _up(bS[i * 320 + p * 64:i * 320 + (p + 1) * 64, :])
        return _dot_nt(_up(xpS[0:hn // 2, i * 256:(i + 1) * 256]), w)

    def bu_rem(hn, p):
        xr = jnp.concatenate([_up(xpS[0:hn // 2, 1792:1920]), _up(xpS[0:hn // 2, 1920:2048])], axis=0)
        w = jnp.concatenate([bcat[p * 128:(p + 1) * 128, 512:640],
                             bcat[D + p * 128:D + (p + 1) * 128, 512:640]], axis=0)
        return _dot_nt(xr, w)

    def bu_fin(m, rem):
        c11, c12, c21, c22 = _combine(m)
        return (jnp.concatenate([c11, c21], axis=0) + rem[:, 0:128],
                jnp.concatenate([c12, c22], axis=0) + rem[:, 128:256])

    u = {}

    def bu_plain(tiles, c0, c1, split=False):
        w = jnp.concatenate([bcat[t * 128:(t + 1) * 128, c0:c1] for t in tiles], axis=0)
        if split:
            r = jnp.concatenate([_dot_nt(_up(xp[0:128, c0:c1]), w),
                                 _dot_nt(_up(xp[128:256, c0:c1]), w)], axis=0)
        else:
            r = _dot_nt(_up(xp[:, c0:c1]), w)
        for i, t in enumerate(tiles):
            u[t] = u[t] + _lt(r, i) if t in u else _lt(r, i)

    carry = {}

    def b_scan(items):
        sub8 = lax.broadcasted_iota(jnp.int32, (8, 128), 0)
        chains = []
        for bu, t0, lt in items:
            for c in range(bu[0].shape[0] // TB):
                for si in range(2):
                    chains.append((bu, c * TB + BASES[si], si, lt, t0))
        lam = {lt: (tab[T_LR, :, lt * 128:(lt + 1) * 128], tab[T_LI, :, lt * 128:(lt + 1) * 128])
               for _, _, lt in items}
        tb = lambda si, k, lt: (tab[_tab_idx(si, k, 0), :, lt * 128:(lt + 1) * 128],
                                tab[_tab_idx(si, k, 1), :, lt * 128:(lt + 1) * 128])
        ld = lambda bu, r: (bu[0][r:r + 8, :], bu[1][r:r + 8, :])

        def step(h, a, b):
            return (a[0] * h[0] - a[1] * h[1] + b[0], a[0] * h[1] + a[1] * h[0] + b[1])

        st = [ld(bu, o) for bu, o, si, lt, t0 in chains]
        for j in range(1, max(SEGS)):
            for ix, (bu, o, si, lt, t0) in enumerate(chains):
                if j < SEGS[si]:
                    st[ix] = step(st[ix], lam[lt], ld(bu, o + 8 * j))
        for k in range(3):
            for ix, (bu, o, si, lt, t0) in enumerate(chains):
                e = st[ix]
                sh = (pltpu.roll(e[0], 1 << k, 0), pltpu.roll(e[1], 1 << k, 0))
                st[ix] = step(sh, tb(si, k, lt), e)
        for ix, (bu, o, si, lt, t0) in enumerate(chains):
            rl = tuple(jnp.where(sub8 == 0, 0.0, pltpu.roll(v, 1, 0)) for v in st[ix])
            prev = carry.get(lt)
            h = rl if prev is None else step(prev, tb(si, 3, lt), rl)
            for j in range(0, SEGS[si], 4):
                r = o + 8 * j
                h1 = step(h, lam[lt], ld(bu, r))
                h2 = step(h1, lam[lt], ld(bu, r + 8))
                h3 = step(h2, lam[lt], ld(bu, r + 16))
                h = step(h3, lam[lt], ld(bu, r + 24))
                cat = lambda a, b: jnp.concatenate([a, b], axis=0)
                a11, a12 = cat(h1[0], h2[0]), cat(h1[1], h2[1])
                a21, a22 = cat(h3[0], h[0]), cat(h3[1], h[1])
                sm = _sums_a(a11, a12, a21, a22)
                rows = pl.ds(quarter(t0) + r // 4, 8)
                for k, v in enumerate([a11, a12, a21, a22, sm[0], sm[1], sm[4], sm[5], sm[6]]):
                    hb[rows, k * D + lt * 128:k * D + (lt + 1) * 128] = _pk(v)
            carry[lt] = tuple(jnp.broadcast_to(v[7:8, :], (8, 128)) for v in h)

    def carry_save():
        for lt in range(NL):
            carry_ref[0, :, lt * 128:(lt + 1) * 128] = carry[lt][0]
            carry_ref[1, :, lt * 128:(lt + 1) * 128] = carry[lt][1]

    def carry_load():
        for lt in range(NL):
            carry[lt] = (carry_ref[0, :, lt * 128:(lt + 1) * 128],
                         carry_ref[1, :, lt * 128:(lt + 1) * 128])

    def y_store(t0, ytop, ybot, lt):
        dv = tab[T_D, :, lt * 128:(lt + 1) * 128]
        for base, n in zip(BASES, SEGS):
            for j in range(0, n, 2):
                xv = b_ld2(t0, base // 8 + j, lt)
                r = (base + 8 * (j - j % 4)) // 2
                y = ytop if j % 4 < 2 else ybot
                for e in range(2):
                    idx = pl.ds(t0 + base + j + e, 8, stride=n)
                    ys[lt, idx, :] = y[r + 8 * e:r + 8 * e + 8, :] + xv[8 * e:8 * e + 8] * dv
        out_b(t0, lt).start()

    hidx = {0: 4, 1: 5, 2: 0, 3: 3, 4: 6, 5: 7, 6: 8}

    def y_main(t0, order=ORD):
        rows = pl.ds(quarter(t0), TB // 4)
        m = [None] * 7
        for i in order:
            m[i] = _dot_nt(_up(hb[rows, hidx[i] * D:(hidx[i] + 1) * D]),
                           _up(cS[i * 128:(i + 1) * 128, :]))
        c11, c12, c21, c22 = _combine(m)
        for c in range(2):
            y_store(t0, _lt(c12, c), _lt(c22, c), 2 + c)
        for c in range(2):
            y_store(t0, _lt(c11, c), _lt(c21, c), c)

    def y_rem(t0):
        rows = pl.ds(quarter(t0), TB // 4)
        h = jnp.concatenate([_up(hb[rows, 0:2 * D]), _up(hb[rows, 2 * D:4 * D])], axis=0)
        y = _dot_nt(h, _up(cR[...]))
        y_store(t0, y[0:128], y[128:256], 4)

    def tables():
        lre = v_lre[...].astype(F32).reshape(1, D)
        lim = v_lim[...].astype(F32).reshape(1, D)
        dt = jnp.exp(v_ldt[...].astype(F32).reshape(1, D)).astype(BF16).astype(F32)
        dsk = v_dsk[...].astype(F32).reshape(1, D)
        mag = jnp.exp(dt * lre)
        ang = dt * lim
        lbr = mag * jnp.cos(ang)
        lbi = mag * jnp.sin(ang)
        sc = jnp.maximum(jnp.abs(lre), jnp.abs(lim))
        a_ = lre / sc
        b_ = lim / sc
        dn = (a_ * a_ + b_ * b_) * sc
        nr = lbr - 1.0
        cr = (nr * a_ + lbi * b_) / dn
        ci = (lbi * a_ - nr * b_) / dn
        bc = lambda v: jnp.broadcast_to(v, (8, D))
        sub = lax.broadcasted_iota(jnp.int32, (8, D), 0)
        tab[T_LR] = bc(lbr)
        tab[T_LI] = bc(lbi)
        tab[T_D] = bc(dsk)
        tab[T_CR] = bc(2.0 * cr)
        tab[T_CI] = bc(2.0 * ci)
        tab[T_NCI] = bc(-2.0 * ci)
        pw = [(lbr, lbi)]
        for _ in range(4):
            pw.append(_cmul(*pw[-1], *pw[-1]))
        for si, n in enumerate(SEGS):
            acc = None
            for b in range(5):
                if (n >> b) & 1:
                    acc = pw[b] if acc is None else _cmul(*acc, *pw[b])
            w = (jnp.ones((8, D), F32), jnp.zeros((8, D), F32))
            for k in range(3):
                a8 = (bc(acc[0]), bc(acc[1]))
                tab[_tab_idx(si, k, 0)] = jnp.where(sub >= (1 << k), a8[0], 0.0)
                tab[_tab_idx(si, k, 1)] = jnp.where(sub >= (1 << k), a8[1], 0.0)
                wm = _cmul(*w, *a8)
                bit = ((sub >> k) & 1) == 1
                w = (jnp.where(bit, wm[0], w[0]), jnp.where(bit, wm[1], w[1]))
                if k < 2:
                    acc = _cmul(*acc, *acc)
            tab[_tab_idx(si, 3, 0)] = w[0]
            tab[_tab_idx(si, 3, 1)] = w[1]

    def c_prep():
        def pq(r, lt, which):
            cs = slice(lt * 128, (lt + 1) * 128)
            c_r = cre[r:r + 16, cs].astype(F32)
            c_i = cim[r:r + 16, cs].astype(F32)
            if which == 0:
                return c_r * tab[T_CR, 0:1, cs] - c_i * tab[T_CI, 0:1, cs]
            return c_r * tab[T_NCI, 0:1, cs] - c_i * tab[T_CR, 0:1, cs]

        def put(i, r, lt, v):
            cS[i * 128 + r // 2:i * 128 + r // 2 + 8, lt * 128:(lt + 1) * 128] = _pk(v)

        p1, q2 = {}, {}
        pos = [(r, lt) for r in range(0, 256, 16) for lt in range(NL)]
        for r, lt in pos:
            p1[r, lt] = pq(r, lt, 0)
            put(1, r, lt, p1[r, lt])
        for r, lt in pos:
            q2[r, lt] = pq(256 + r, lt, 1)
            put(4, r, lt, q2[r, lt])
            put(0, r, lt, p1[r, lt] + q2[r, lt])
        for r, lt in pos:
            q1 = pq(r, lt, 1)
            put(3, r, lt, q1 - p1[r, lt])
            put(6, r, lt, q1 + q2[r, lt])
        for r, lt in pos:
            p2 = pq(256 + r, lt, 0)
            put(2, r, lt, p2 - q2[r, lt])
            put(5, r, lt, p1[r, lt] + p2)
        for which in range(2):
            for r in range(0, 128, 16):
                for lt in range(NL):
                    cR[r // 2:r // 2 + 8, which * D + lt * 128:which * D + (lt + 1) * 128] = _pk(
                        pq(512 + r, lt, which))

    def wk_prep():
        blk = lambda kt, ft: wk[kt * 128:(kt + 1) * 128, ft * 128:(ft + 1) * 128].astype(F32)
        rnd = lambda v: v.astype(BF16).astype(F32)
        for i in ORDK:
            for fp in range(2):
                for c in range(2):
                    v = _op_b(i, lambda kh, nh: blk(2 * kh + c, 2 * fp + nh))
                    wkS[i * 160 + fp * 64:i * 160 + (fp + 1) * 64, c * 128:(c + 1) * 128] = _pk(rnd(v).T)
        for c in range(2):
            t = [blk(c, 4).T, blk(2 + c, 4).T]
            for i in range(7):
                v = _op_b(i, lambda kh, nh: t[kh][64 * nh:64 * (nh + 1)])
                wkS[i * 160 + 128:i * 160 + 160, c * 128:(c + 1) * 128] = _pk(v)
        pos = 0
        tr = [blk(4, ft).T for ft in range(NL)]
        for lo, hi in KTOP + KBOT:
            wkR[pos // 2:(pos + hi - lo) // 2, :] = _pk(tr[lo // 128][lo % 128:lo % 128 + hi - lo])
            pos += hi - lo

    def wq_transpose():
        for lt in range(NL):
            slab2[lt] = wq[lt * 128:(lt + 1) * 128, :].astype(F32).T

    def wq_ops():
        g = lambda d, lt: slab2[lt, pl.ds(d, H, stride=DH), :]
        for i in ORD:
            for d in range(8):
                for c in range(2):
                    v = _op_b(i, lambda kh, nh: g(d + 8 * nh, 2 * kh + c))
                    wqS[i * 128 + d * 16:i * 128 + (d + 1) * 16, c * 128:(c + 1) * 128] = _pk(v)
        for d in range(16):
            wqKR[d * 16:(d + 1) * 16, :] = _pk(g(d, 4))
        for d in range(16, 20):
            for lt in range(NL):
                wqNR[(d - 16) * 16:(d - 15) * 16, lt * 128:(lt + 1) * 128] = _pk(g(d, lt))

    xidx = {0: 0, 1: 1, 4: 2, 5: 3, 6: 4}

    def x_sums(a0):
        for r in range(0, 256, 32):
            for c in range(2):
                g = lambda ro, co: xa[pl.ds(a0 + ro + r, 32),
                                      (co + c) * 128:(co + c + 1) * 128].astype(F32)
                sm = _sums_a(g(0, 0), g(0, 2), g(256, 0), g(256, 2))
                for i, k in xidx.items():
                    xS[k * 128 + r // 2:k * 128 + r // 2 + 16, c * 128:(c + 1) * 128] = _pk(sm[i])

    def x_op(a0, i):
        if i == 2:
            return xa[pl.ds(a0, 256), 0:256]
        if i == 3:
            return xa[pl.ds(a0 + 256, 256), 256:512]
        return _up(xS[xidx[i] * 128:(xidx[i] + 1) * 128, :])

    def a_k(a0):
        rem = _dot_nt(_up(wkR[...]), xa[pl.ds(a0, 512), 512:640])
        m = [None] * 7
        for i in ORDK:
            m[i] = _dot_nt(_up(wkS[i * 160:(i + 1) * 160, :]), x_op(a0, i))
        c11, c12, c21, c22 = _combine(m)
        a11 = _phi(c11 + rem[0:320, 0:256])
        a12 = _phi(c21 + rem[0:320, 256:512])
        a21 = _phi(c12 + rem[320:640, 0:256])
        a22 = _phi(c22 + rem[320:640, 256:512])
        zt = (_lt(a11, 0) + _lt(a11, 1)) + (_lt(a12, 0) + _lt(a12, 1))
        zb = (_lt(a21, 0) + _lt(a21, 1)) + (_lt(a22, 0) + _lt(a22, 1))
        for zz, rngs in ((zt, KTOP), (zb, KBOT)):
            pos = 0
            for lo, hi in rngs:
                zacc[lo:hi, :] += zz[pos:pos + hi - lo]
                pos += hi - lo
        ops = [v.astype(BF16) for v in _sums_a(a11, a12, a21, a22)]
        full = jnp.concatenate([jnp.concatenate([ops[2], a12.astype(BF16)], axis=1),
                                jnp.concatenate([a21.astype(BF16), ops[3]], axis=1)], axis=0)
        return ops, full

    gmap = {0: 0, 1: 2, 2: 6, 3: 5, 4: 3, 5: 4, 6: 1}

    def a_q_nrem(a0):
        pqs[pl.ds(a0, 512), 512:640] = _phi(_dot_nt(xa[pl.ds(a0, 512), :], _up(wqNR[...])))

    def a_q(a0):
        rem = _dot_nt(xa[pl.ds(a0, 512), 512:640], _up(wqKR[...]))
        m = [None] * 7
        for i in ORDK:
            m[i] = _dot_nt(x_op(a0, i), _up(wqS[i * 128:(i + 1) * 128, :]))
        c11, c12, c21, c22 = _combine(m)
        pqs[pl.ds(a0, 256), 0:256] = _phi(c11 + rem[0:256, 0:256])
        pqs[pl.ds(a0, 256), 256:512] = _phi(c12 + rem[0:256, 256:512])
        pqs[pl.ds(a0 + 256, 256), 0:256] = _phi(c21 + rem[256:512, 0:256])
        pqs[pl.ds(a0 + 256, 256), 256:512] = _phi(c22 + rem[256:512, 256:512])

    def a_z():
        for lt in range(NL):
            zp = jnp.concatenate(
                [zacc[pl.ds(d, H, stride=DH), :] for d in range(4 * lt, 4 * lt + 4)], axis=0)
            zrow[:, lt * 128:(lt + 1) * 128] = jnp.broadcast_to(
                jnp.sum(zp.T, axis=0, keepdims=True), (8, 128))

    def g_pack(gm, gr):
        c11, c12, c21, c22 = _combine(gm)
        for top, (cl, cr_), rngs in ((0, (c11, c12), KTOP), (320, (c21, c22), KBOT)):
            pos = 0
            for lo, hi in rngs:
                gb[lo // 2:hi // 2, 0:256] = _pk(cl[pos:pos + hi - lo])
                gb[lo // 2:hi // 2, 256:512] = _pk(cr_[pos:pos + hi - lo])
                gb[lo // 2:hi // 2, 512:640] = _pk(gr[top + pos:top + pos + hi - lo])
                pos += hi - lo

    def a_kv():
        for j, (lo, hi) in enumerate(KVR):
            kv = _dot(_up(gb[lo // 2:hi // 2, :]), wv[:, j * 128:(j + 1) * 128])
            rh = (lax.broadcasted_iota(jnp.int32, kv.shape, 0) + lo) // DH
            ch = (lax.broadcasted_iota(jnp.int32, kv.shape, 1) + j * 128) // DH
            kvs[j * 80:j * 80 + (hi - lo) // 2, :] = _pk(jnp.where(rh == ch, kv, 0.0))

    def a_m():
        parts = [_dot(_up(kvs[j * 80:j * 80 + (hi - lo) // 2, :]), wo[j * 128:(j + 1) * 128, :])
                 for j, (lo, hi) in enumerate(KVR)]
        pieces = []
        pos = 0
        for j, (lo, hi) in enumerate(KVR):
            nxt = KVR[j + 1][0] if j + 1 < len(KVR) else hi
            pieces.append(parts[j][pos - lo:nxt - lo])
            if j + 1 < len(KVR):
                pieces.append(parts[j][nxt - lo:hi - lo] + parts[j + 1][0:hi - nxt])
                pos = hi
        m = jnp.concatenate(pieces, axis=0)
        for lt in range(NL):
            slab[lt] = _lt(m, lt)
        g = lambda d, lt: slab[lt, pl.ds(d, H, stride=DH), :]
        for i in ORD:
            for d in range(8):
                for c in range(2):
                    v = _op_b(i, lambda kh, nh: g(d + 8 * kh, 2 * nh + c))
                    mS[i * 128 + d * 16:i * 128 + (d + 1) * 16, c * 128:(c + 1) * 128] = _pk(v)
        for d in range(16, 20):
            for lt in range(4):
                mKR[(d - 16) * 16:(d - 15) * 16, lt * 128:(lt + 1) * 128] = _pk(g(d, lt))
        for d in range(DH):
            mNR[d * 16:(d + 1) * 16, :] = _pk(g(d, 4))

    def a_o(a0, n):
        hn = n // 2
        for r in range(a0, a0 + n, NB):
            t = pqs[r:r + NB, 0:128] * zrow[0:1, 0:128]
            for lt in range(1, NL):
                t = t + pqs[r:r + NB, lt * 128:(lt + 1) * 128] * zrow[0:1, lt * 128:(lt + 1) * 128]
            t = t + pltpu.roll(t, 64, 1)
            t = t + pltpu.roll(t, 32, 1)
            rrs[r:r + NB, :] = 1.0 / (t + 1e-6)

        def norm_rows(r):
            pq = pqs[r:r + NB, :]
            rr = rrs[r:r + NB, :]
            return jnp.concatenate([_lt(pq, lt) * rr for lt in range(NL)], axis=1)

        tops, bots, sums = [], [], [[] for _ in range(7)]
        for r in range(0, hn, NB):
            tp = norm_rows(a0 + r)
            bt = norm_rows(a0 + hn + r)
            sm = _sums_a(tp[:, 0:256], tp[:, 256:512], bt[:, 0:256], bt[:, 256:512])
            tops.append(tp.astype(BF16))
            bots.append(bt.astype(BF16))
            for i in (0, 1, 4, 5, 6):
                sums[i].append(sm[i].astype(BF16))
        full = jnp.concatenate(tops + bots, axis=0)
        ops = [None] * 7
        for i in (0, 1, 4, 5, 6):
            ops[i] = jnp.concatenate(sums[i], axis=0)
        ops[2] = full[0:hn, 0:256]
        ops[3] = full[hn:n, 256:512]
        oa[a0:a0 + n, 512:640] = _dot(full, _up(mNR[...]))
        rem = _dot(full[:, 512:640], _up(mKR[...]))
        m = [None] * 7
        for i in ORD:
            m[i] = _dot(ops[i], _up(mS[i * 128:(i + 1) * 128, :]))
        c11, c12, c21, c22 = _combine(m)
        oa[a0:a0 + hn, 0:256] = c11 + rem[0:hn, 0:256]
        oa[a0:a0 + hn, 256:512] = c12 + rem[0:hn, 256:512]
        oa[a0 + hn:a0 + n, 0:256] = c21 + rem[hn:n, 0:256]
        oa[a0 + hn:a0 + n, 256:512] = c22 + rem[hn:n, 256:512]
        out_a(a0, n).start()

    gM[...] = jnp.zeros(gM.shape, F32)
    gR[...] = jnp.zeros(gR.shape, F32)
    zacc[...] = jnp.zeros(zacc.shape, F32)
    wait(6)
    tables()

    def sc(ps):
        b_scan([((u.pop(p), u.pop(p + 5)), 0, p) for p in ps])

    wait(0)
    b_prep(0, [0, 1])
    b_prep(256, [0, 1])
    bu_plain(range(N0), 0, 256, True)
    wait(1)
    bu_plain(range(N0, 10), 0, 256, True)
    wait(2)
    b_prep(0, [2, 3, 4])
    b_prep(256, [2, 3, 4])
    bu_plain([0, 5], 256, D)
    sc([0])
    bu_plain([1, 6], 256, D)
    sc([1])
    bu_plain([2, 3], 256, D, True)
    wait(3)
    bu_plain([7, 8], 256, D)
    sc([2, 3])
    bu_plain([4, 9], 256, D)
    sc([4])

    b_stage(512)
    b_stage(768)
    hn = b_prep_s([(512, g) for g in range(0, 32, 2)], [(768, g) for g in range(0, 32, 2)])
    mt = {}

    def rem1(p):
        mt[p] = ([None] * 7, bu_rem(hn, p))

    def prod1(p, k0, k1):
        for k in range(k0, k1):
            bs_op(p, ORD[k])
            mt[p][0][ORD[k]] = bu_prod(hn, p, ORD[k])
        if k1 == 7:
            b_scan([(bu_fin(*mt[p]), 512, p)])

    rem1(0)
    rem1(1)
    rem1(2)
    prod1(0, 0, 7)
    prod1(1, 0, 7)
    prod1(2, 0, 7)
    rem1(3)
    prod1(3, 0, 3)
    wait(4)
    c_prep()
    prod1(3, 3, 5)
    rem1(4)
    y_main(0, ORDY0)
    prod1(3, 5, 7)
    prod1(4, 0, 7)
    y_main(TB)
    y_rem(0)
    y_rem(TB)
    carry_save()
    wk_prep()
    wq_transpose()

    def main(i, c):
        for cc in it_copies(i):
            cc.wait()
        a0 = pl.multiple_of(i * 512, 512)
        tb0 = chunk(i + 4)
        ty = chunk(i + 2)
        b_stage(tb0)
        x_sums(a0)
        wq_ops()
        y_rem(ty)
        ops, full = a_k(a0)
        a_q_nrem(a0)
        h2 = b_prep_s([(tb0, g) for g in range(0, 16, 2)], [(tb0, g) for g in range(16, 32, 2)])
        carry_load()
        for p in range(NL):
            rem = bu_rem(h2, p)
            m = [None] * 7
            for k in ORD:
                m[k] = bu_prod(h2, p, k)
            b_scan([(bu_fin(m, rem), tb0, p)])
        carry_save()
        gm = [None] * 7
        for k in ORDG:
            gm[k] = gM[k] + _dot(ops[k], x_op(a0, gmap[k]))
            gM[k] = gm[k]
        a_q(a0)
        y_main(ty)
        gr = gR[...] + _dot(full, xa[pl.ds(a0, 512), 512:640])
        gR[...] = gr
        g_pack(gm, gr)
        a_z()
        return c

    lax.fori_loop(0, 4, main, 0)

    wait(5)
    a_kv()
    y_main(6 * TB)
    a_m()
    y_rem(6 * TB)
    for i in range(8):
        a_o(i * 256, 256)
    y_main(7 * TB)
    y_rem(7 * TB)

    for c in range(8):
        for lt in range(NL):
            out_b(c * TB, lt).wait()
    for i in range(8):
        out_a(i * 256, 256).wait()


def _compiler_params():
    base = dict(vmem_limit_bytes=110 * 1024 * 1024)
    for extra in (dict(disable_bounds_checks=True, disable_semaphore_checks=True),
                  dict(disable_bounds_checks=True), dict()):
        try:
            return pltpu.CompilerParams(**base, **extra)
        except TypeError:
            continue
    return None


@jax.jit
def pallas_concat_heads__linear_attn_block__ssm_conv_s5__prompt_kernel(
    A_x: jax.Array,
    A_wqkv: jax.Array,
    A_wo: jax.Array,
    B_x: jax.Array,
    B_Lambda_re: jax.Array,
    B_Lambda_im: jax.Array,
    B_B_re: jax.Array,
    B_B_im: jax.Array,
    B_C_re: jax.Array,
    B_C_im: jax.Array,
    B_log_dt: jax.Array,
    B_Dskip: jax.Array,
):
    any_spec = pl.BlockSpec(memory_space=pl.ANY)
    V = pltpu.VMEM
    return pl.pallas_call(
        _kernel,
        out_shape=jax.ShapeDtypeStruct((1, S, 2 * D), F32),
        in_specs=[any_spec] * 12,
        out_specs=any_spec,
        scratch_shapes=[
            V((S, D), BF16),
            V((S, D), BF16),
            V((NL * (S // 2), 128), U32),
            V((D, D), BF16),
            V((D, D), BF16),
            V((D, D), BF16),
            V((D, D), BF16),
            V((2 * D, D), BF16),
            V((D, D), BF16),
            V((D, D), BF16),
            V((7 * 128, D), U32),
            V((64, 2 * D), U32),
            V((NL, D, 128), F32),
            V((NL, D, 128), F32),
            V((NTAB, 8, D), F32),
            V((256, D), U32),
            V((S // 4, 9 * D), U32),
            V((NL, S, 128), F32),
            V((S, D), F32),
            V((7, 320, 256), F32),
            V((D, 128), F32),
            V((D, 128), F32),
            V((NL * 80, 128), U32),
            V((7 * 128, 256), U32),
            V((64, 512), U32),
            V((320, 128), U32),
            V((8, D), F32),
            V((2, 8, D), F32),
            V((S, D), F32),
            V((7 * 160, 256), U32),
            V((320, 128), U32),
            V((7 * 128, 256), U32),
            V((256, 128), U32),
            V((64, D), U32),
            V((5 * 128, 256), U32),
            V((128, 2048), U32),
            V((7 * 320, 256), U32),
            V((S, 128), F32),
            V((D // 2, D), U32),
            V((D,), BF16), V((D,), BF16), V((D,), BF16), V((D,), BF16),
            pltpu.SemaphoreType.DMA((11,)),
            pltpu.SemaphoreType.DMA((1,)),
        ],
        compiler_params=_compiler_params(),
    )(A_x, A_wqkv, A_wo, B_x, B_Lambda_re, B_Lambda_im, B_B_re, B_B_im,
      B_C_re, B_C_im, B_log_dt, B_Dskip)
```
